```python
import jax
import jax.numpy as jnp

def _softmax(x, axis=-1):
    return jax.nn.softmax(x, axis=axis)
def _gelu(x):
    return jax.nn.gelu(x, approximate=True)
def _silu(x):
    return jax.nn.silu(x)
def _sigmoid(x):
    return jax.nn.sigmoid(x)
def _layernorm(x, axis=-1, eps=1e-5):
    m = jnp.mean(x, axis=axis, keepdims=True)
    v = jnp.var(x, axis=axis, keepdims=True)
    return (x - m) / jnp.sqrt(v + eps)
def _scatter_add(tgt, idx, src, axis=0):
    return tgt.at[idx].add(src)
def _segment_sum(src, seg, n):
    return jax.ops.segment_sum(src, seg, n)
class _Rng:
    def __init__(self, key):
        self._k = key
    def _next(self):
        self._k, sub = jax.random.split(self._k)
        return sub
    def normal(self, shape):
        return jax.random.normal(self._next(), shape, dtype=jnp.bfloat16)
    def randint(self, lo, hi, shape):
        return jax.random.randint(self._next(), shape, lo, hi, dtype=jnp.int32)
    def uniform(self, shape, lo=0.0, hi=1.0):
        return jax.random.uniform(self._next(), shape, jnp.bfloat16, lo, hi)
    def permutation(self, n):
        return jax.random.permutation(self._next(), n)


kernel_name = 'parallel_sum__ssm_conv_h3__dense_activation_gelu__prompt'

def setup_inputs():
    _rng = _Rng(jax.random.key(int.from_bytes(__import__("os").urandom(4), "little")))
    _w = (lambda a: (lambda t: t.astype(jnp.bfloat16) if jnp.issubdtype(t.dtype, jnp.floating) else t)(jnp.asarray(a)))
    def _A_setup():
        B, S, D = 1, 2048, 640
        ks = 4
        return {
            "q": _w((lambda *s: _rng.normal(s) * 0.05)(B, S, D)),
            "k": _w((lambda *s: _rng.normal(s) * 0.05)(B, S, D)),
            "v": _w((lambda *s: _rng.normal(s) * 0.05)(B, S, D)),
            "shift_k": _w((lambda *s: _rng.normal(s) * 0.05)(D, ks) * 0.5),
            "ssm_k": _w((lambda *s: _rng.normal(s) * 0.05)(D, S) * (1.0 / S ** 0.5)),
            "ssm_D": _w((lambda *s: _rng.normal(s) * 0.05)(D)),
        }
    _A_in = _A_setup()

    def _B_setup():
        B, S, D, F = 1, 2048, 640, 1728
        return {
            "x": _w((lambda *s: _rng.normal(s) * 0.05)(B, S, D)),
            "w1": _w((lambda *s: _rng.normal(s) * 0.05)(D, F) * (D ** -0.5)),
            "b1": _w((lambda *s: _rng.normal(s) * 0.05)(F) * 0.01),
            "w2": _w((lambda *s: _rng.normal(s) * 0.05)(F, D) * (F ** -0.5)),
            "b2": _w((lambda *s: _rng.normal(s) * 0.05)(D) * 0.01),
        }
    _B_in = _B_setup()

    return {
        "A_q": _A_in["q"],
        "A_k": _A_in["k"],
        "A_v": _A_in["v"],
        "A_shift_k": _A_in["shift_k"],
        "A_ssm_k": _A_in["ssm_k"],
        "A_ssm_D": _A_in["ssm_D"],
        "B_x": _B_in["x"],
        "B_w1": _B_in["w1"],
        "B_b1": _B_in["b1"],
        "B_w2": _B_in["w2"],
        "B_b2": _B_in["b2"],
    }

def reference(A_q, A_k, A_v, A_shift_k, A_ssm_k, A_ssm_D, B_x, B_w1, B_b1, B_w2, B_b2):
    def _A_ref(q, k, v, shift_k, ssm_k, ssm_D):
        B, S, D = q.shape
        ks = shift_k.shape[-1]
        k_pad = jnp.pad(k, ((0, 0), (ks - 1, 0), (0, 0)))
        k_shift = jnp.zeros_like(k)
        for t in range(ks):
            k_shift = k_shift + k_pad[:, t:t + S, :] * shift_k[:, ks - 1 - t][None, None, :]
        kv = k_shift * v
        L = 2 * S
        kv_pad = jnp.pad(kv, ((0, 0), (0, S), (0, 0)))
        kf_pad = jnp.pad(ssm_k, ((0, 0), (0, S)))
        kv_f = (lambda x, axes=(-2,-1): jnp.fft.rfft2(x.astype(jnp.float32), axes=axes))(kv_pad[:, None, :, :], axes=(1, 2))
        kf_f = (lambda x, axes=(-2,-1): jnp.fft.rfft2(x.astype(jnp.float32), axes=axes))(kf_pad[:, None, :], axes=(1, 2))
        kf_f = (lambda x, *d: x.transpose(*d))(kf_f, 1, 2, 0)
        y_f = kv_f * kf_f[None, :, :, :]
        y = (lambda x, s, axes=(-2,-1): jnp.fft.irfft2(x, s=s, axes=axes).astype(jnp.bfloat16))(y_f, (1, L), axes=(1, 2))[:, 0, :S, :]
        y = y + kv * ssm_D[None, None, :]
        return q * y

    def _B_ref(x, w1, b1, w2, b2):
        h = jnp.einsum("bsd,df->bsf", x, w1) + b1
        h = _gelu(h)
        return jnp.einsum("bsf,fd->bsd", h, w2) + b2

    x = A_q
    xn = _layernorm(x, axis=-1)
    return x + _A_ref(xn, A_k, A_v, A_shift_k, A_ssm_k, A_ssm_D) + _B_ref(xn, B_w1, B_b1, B_w2, B_b2)
```

```python
import jax
import jax.numpy as jnp
import numpy as np
import jax.experimental.pallas as pl
import jax.experimental.pallas.tpu as pltpu

S, D, F, KS = 2048, 640, 1728, 4
N1, N2 = 128, 16
G = D // 128
BM = 256
NB = S // BM
bf16, f32, u32 = jnp.bfloat16, jnp.float32, jnp.uint32


def _dft_mats():
    k1 = np.arange(N1)[None, :, None]
    n1 = np.arange(N1)[None, None, :]
    n2 = np.arange(N2)[:, None, None]
    ang = -2.0 * np.pi * (k1 + 0.25) * (N2 * n1 + n2) / S
    fr, fi = np.cos(ang), np.sin(ang)
    fwd = np.concatenate([fr, fi], axis=1)
    inv = np.stack([fr, fi], axis=2).reshape(N2, 2 * N1, N1)
    inv = np.transpose(inv, (0, 2, 1)) / S
    return fwd.astype(jnp.bfloat16), inv.astype(jnp.bfloat16)


_FWD, _INV = _dft_mats()

_C1, _S1, _R2 = float(np.cos(np.pi / 8)), float(np.sin(np.pi / 8)), float(np.sqrt(0.5))


def _bf4(a, b, c, d, sgn):
    t0 = (a[0] + c[0], a[1] + c[1])
    t1 = (a[0] - c[0], a[1] - c[1])
    t2 = (b[0] + d[0], b[1] + d[1])
    t3 = (b[0] - d[0], b[1] - d[1])
    o0 = (t0[0] + t2[0], t0[1] + t2[1])
    o2 = (t0[0] - t2[0], t0[1] - t2[1])
    p = (t1[0] + t3[1], t1[1] - t3[0])
    q = (t1[0] - t3[1], t1[1] + t3[0])
    return (o0, p, o2, q) if sgn < 0 else (o0, q, o2, p)


def _tw(x, e, sgn):
    r, i = x
    if e == 0:
        return x
    if e == 4:
        return (i, -r) if sgn < 0 else (-i, r)
    if e == 2:
        return ((r + i) * _R2, (i - r) * _R2) if sgn < 0 else ((r - i) * _R2, (r + i) * _R2)
    if e == 6:
        return ((i - r) * _R2, (r + i) * -_R2) if sgn < 0 else ((r + i) * -_R2, (r - i) * _R2)
    c = float(np.cos(2 * np.pi * e / 16))
    s = sgn * float(np.sin(2 * np.pi * e / 16))
    return (r * c - i * s, r * s + i * c)


def _fft16(x, sgn):
    y = [[None] * 4 for _ in range(4)]
    for b in range(4):
        o = _bf4(x[b], x[4 + b], x[8 + b], x[12 + b], sgn)
        for c in range(4):
            y[c][b] = _tw(o[c], b * c, sgn)
    out = [None] * 16
    for c in range(4):
        o = _bf4(y[c][0], y[c][1], y[c][2], y[c][3], sgn)
        for d in range(4):
            out[c + 4 * d] = o[d]
    return out


def _lo(w):
    return pltpu.bitcast(w << 16, f32)


def _hi(w):
    return pltpu.bitcast(w & u32(0xFFFF0000), f32)


def _pack(a, b):
    return pltpu.pack_elementwise([a, b], packed_dtype=bf16).astype(u32)


def _gelu(h):
    c1 = 0.7978845608028654
    u = h * (c1 + (c1 * 0.044715) * (h * h))
    hh = 0.5 * h
    return hh + hh * jnp.tanh(u)


def _kernel(q_hbm, k_hbm, v_hbm, sk_ref, ssm_hbm, d_ref, w1_hbm, b1_ref, w2_hbm, b2_ref,
            fwd_hbm, inv_hbm, o_hbm,
            q_buf, k_buf, v_buf, ssm_buf, w1_buf, w2_buf, fwd_buf, inv_buf,
            kt_buf, rhs_buf, ya, yb, z_buf, y_buf, xn_buf, acc, o_buf, sems):
    cps = {}

    def start(name, src, dst):
        cp = pltpu.make_async_copy(src, dst, sems.at[len(cps)])
        cp.start()
        cps[name] = cp

    start("q", q_hbm.at[0], q_buf)
    start("w1", w1_hbm, w1_buf)
    start("w2", w2_hbm, w2_buf)
    for g in range(G):
        ls = pl.ds(g * 128, 128)
        start(("k", g), k_hbm.at[0, :, ls], k_buf.at[g, pl.ds(16, S)])
        start(("v", g), v_hbm.at[0, :, ls], v_buf.at[g])
    start("ssm", ssm_hbm, ssm_buf)
    start("fwd", fwd_hbm, fwd_buf)
    start("inv", inv_hbm, inv_buf)

    kw = k_buf.bitcast(u32)
    vw = v_buf.bitcast(u32)
    ktw = kt_buf.bitcast(u32)

    def mlp(i):
        r = pl.ds(pl.multiple_of(i * BM, BM), BM)
        x = q_buf[r, :].astype(f32)
        m = jnp.mean(x, axis=-1, keepdims=True)
        xc = x - m
        var = jnp.mean(xc * xc, axis=-1, keepdims=True)
        xn = (xc * jax.lax.rsqrt(var + 1e-5)).astype(bf16)
        xn_buf[r, :] = xn
        h = jax.lax.dot_general(xn, w1_buf[...], (((1,), (1,)), ((), ())),
                                preferred_element_type=f32)
        h = _gelu(h + b1_ref[...].astype(f32).reshape(1, F)).astype(bf16)
        o = jnp.dot(h, w2_buf[...], preferred_element_type=f32)
        acc[r, :] = o + (x + b2_ref[...].astype(f32).reshape(1, D))

    def prep(g):
        ls = pl.ds(g * 128, 128)
        k_buf[g, pl.ds(0, 16), :] = jnp.zeros((16, 128), bf16)
        sk = sk_ref[:, ls].astype(f32)
        sk = [jnp.broadcast_to(sk[j:j + 1, :], (8, 128)) for j in range(KS)]
        kt_buf[g] = ssm_buf[ls, :].T
        dd = d_ref[...].astype(f32).reshape(1, D)[:, g * 128:(g + 1) * 128]
        row = jax.lax.broadcasted_iota(jnp.int32, (8, 128), 0)
        dd = jnp.where(row == 0, jnp.broadcast_to(dd, (8, 128)), 0.0)

        def body(a, c):
            res = []
            a128 = pl.multiple_of(a * 128, 128)
            kwa = kw.at[g, pl.ds(a128, 136)]
            vwa = vw.at[g, pl.ds(a128, 128)]
            ktwa = ktw.at[g, pl.ds(a128, 128)]
            for hf in range(2):
                base = hf * 64
                ks = []
                for m in range(-2, 8):
                    w = kwa[pl.ds(base + 8 + m, 8, stride=8), :]
                    ks += [_lo(w), _hi(w)]
                kv = []
                for m in range(8):
                    w = vwa[pl.ds(base + m, 8, stride=8), :]
                    for p, vv in enumerate((_lo(w), _hi(w))):
                        n = 4 + 2 * m + p
                        s = (ks[n] * sk[0] + ks[n - 1] * sk[1]) + (ks[n - 2] * sk[2] + ks[n - 3] * sk[3])
                        kv.append(s * vv)
                kk = []
                for m in range(8):
                    w = ktwa[pl.ds(base + m, 8, stride=8), :]
                    kk += [_lo(w), _hi(w)]
                if hf == 0:
                    kk[0] = kk[0] + jnp.where(a == 0, dd, 0.0)
                res.append((kv, kk))
            r = pl.ds(pl.multiple_of(a * 8, 8), 8)
            for n in range(N2):
                rhs_buf[g, n, r, 0:128] = _pack(res[0][0][n], res[1][0][n])
                rhs_buf[g, n, r, 128:256] = _pack(res[0][1][n], res[1][1][n])
            return c

        jax.lax.fori_loop(0, 8, body, 0)

    def stage1(g):
        def body(n, c):
            rhs = pltpu.bitcast(rhs_buf[g, n], bf16)
            y = jnp.dot(fwd_buf[n], rhs, preferred_element_type=f32)
            ya[g, n] = y[:, 0:128]
            yb[g, n] = y[:, 128:256]
            return c

        jax.lax.fori_loop(0, N2, body, 0)

    def middle(u):
        g = u // 16
        a = pl.multiple_of((u % 16) * 8, 8)
        xa = [(ya[g, n, pl.ds(a, 8), :], ya[g, n, pl.ds(N1 + a, 8), :]) for n in range(N2)]
        xb = [(yb[g, n, pl.ds(a, 8), :], yb[g, n, pl.ds(N1 + a, 8), :]) for n in range(N2)]
        fa = _fft16(xa, -1)
        fb = _fft16(xb, -1)
        c = [(p[0] * q[0] - p[1] * q[1], p[0] * q[1] + p[1] * q[0]) for p, q in zip(fa, fb)]
        z = _fft16(c, 1)
        for n in range(N2):
            z_buf[g, n, pl.ds(a, 8), :] = _pack(z[n][0], z[n][1])

    def inverse(g):
        def body(m, c):
            y0 = jnp.dot(inv_buf[2 * m], pltpu.bitcast(z_buf[g, 2 * m], bf16),
                         preferred_element_type=f32)
            y1 = jnp.dot(inv_buf[2 * m + 1], pltpu.bitcast(z_buf[g, 2 * m + 1], bf16),
                         preferred_element_type=f32)
            y_buf[g, pl.ds(m, N1, stride=8), :] = _pack(y0, y1)
            return c

        jax.lax.fori_loop(0, N2 // 2, body, 0)

    def final(i):
        r = pl.ds(pl.multiple_of(i * BM, BM), BM)
        rw = pl.ds(pl.multiple_of(i * (BM // 2), BM // 2), BM // 2)
        for g in range(G):
            ls = pl.ds(g * 128, 128)
            y = pltpu.bitcast(y_buf[g, rw, :], bf16).astype(f32)
            o_buf[r, ls] = (acc[r, ls] + xn_buf[r, ls].astype(f32) * y).astype(bf16)

    for n in ("q", "w1", "w2"):
        cps[n].wait()
    pl.loop(0, NB)(mlp)
    cps["ssm"].wait()
    cps["fwd"].wait()
    for g in range(G):
        cps[("k", g)].wait()
        cps[("v", g)].wait()
        prep(g)
        stage1(g)
    pl.loop(0, G * 16)(middle)
    cps["inv"].wait()
    for g in range(G):
        inverse(g)
    pl.loop(0, NB)(final)
    cp = pltpu.make_async_copy(o_buf, o_hbm.at[0], sems.at[len(cps)])
    cp.start()
    cp.wait()


def _perm_fwd():
    r = np.arange(N1)
    n1 = 16 * (r // 16) + 8 * (r % 2) + (r % 16) // 2
    return np.ascontiguousarray(_FWD[:, :, n1])


_FWD_P = _perm_fwd()


@jax.jit
def pallas_parallel_sum__ssm_conv_h3__dense_activation_gelu__prompt_kernel(
    A_q, A_k, A_v, A_shift_k, A_ssm_k, A_ssm_D, B_x, B_w1, B_b1, B_w2, B_b2,
):
    hbm = pl.BlockSpec(memory_space=pl.ANY)
    vmem = pl.BlockSpec(memory_space=pltpu.VMEM)
    return pl.pallas_call(
        _kernel,
        out_shape=jax.ShapeDtypeStruct((1, S, D), bf16),
        in_specs=[hbm, hbm, hbm, vmem, hbm, vmem, hbm, vmem, hbm, vmem, hbm, hbm],
        out_specs=hbm,
        scratch_shapes=[
            pltpu.VMEM((S, D), bf16),
            pltpu.VMEM((G, S + 16, 128), bf16),
            pltpu.VMEM((G, S, 128), bf16),
            pltpu.VMEM((D, S), bf16),
            pltpu.VMEM((F, D), bf16),
            pltpu.VMEM((F, D), bf16),
            pltpu.VMEM((N2, 2 * N1, N1), bf16),
            pltpu.VMEM((N2, N1, 2 * N1), bf16),
            pltpu.VMEM((G, S, 128), bf16),
            pltpu.VMEM((G, N2, N1 // 2, 256), u32),
            pltpu.VMEM((G, N2, 2 * N1, 128), f32),
            pltpu.VMEM((G, N2, 2 * N1, 128), f32),
            pltpu.VMEM((G, N2, N1, 128), u32),
            pltpu.VMEM((G, S // 2, 128), u32),
            pltpu.VMEM((S, D), bf16),
            pltpu.VMEM((S, D), f32),
            pltpu.VMEM((S, D), bf16),
            pltpu.SemaphoreType.DMA((24,)),
        ],
        compiler_params=pltpu.CompilerParams(vmem_limit_bytes=100 * 2**20),
    )(A_q, A_k, A_v, A_shift_k.T, A_ssm_k, A_ssm_D, B_w1.T, B_b1, B_w2, B_b2, _FWD_P, _INV)
```

```python
import jax
import jax.numpy as jnp
import numpy as np
import jax.experimental.pallas as pl
import jax.experimental.pallas.tpu as pltpu

S, D, F, KS = 2048, 640, 1728, 4
N1, N2 = 128, 16
G = D // 128
BM = 256
NB = S // BM
bf16, f32, u32 = jnp.bfloat16, jnp.float32, jnp.uint32


def _dft_mats():
    k1 = np.arange(N1)[None, :, None]
    n1 = np.arange(N1)[None, None, :]
    n2 = np.arange(N2)[:, None, None]
    ang = -2.0 * np.pi * (k1 + 0.25) * (N2 * n1 + n2) / S
    fr, fi = np.cos(ang), np.sin(ang)
    fwd = np.concatenate([fr, fi], axis=1)
    inv = np.stack([fr, fi], axis=2).reshape(N2, 2 * N1, N1)
    inv = np.transpose(inv, (0, 2, 1)) / S
    return fwd.astype(jnp.bfloat16), inv.astype(jnp.bfloat16)


_FWD, _INV = _dft_mats()

_C1, _S1, _R2 = float(np.cos(np.pi / 8)), float(np.sin(np.pi / 8)), float(np.sqrt(0.5))


def _bf4(a, b, c, d, sgn):
    t0 = (a[0] + c[0], a[1] + c[1])
    t1 = (a[0] - c[0], a[1] - c[1])
    t2 = (b[0] + d[0], b[1] + d[1])
    t3 = (b[0] - d[0], b[1] - d[1])
    o0 = (t0[0] + t2[0], t0[1] + t2[1])
    o2 = (t0[0] - t2[0], t0[1] - t2[1])
    p = (t1[0] + t3[1], t1[1] - t3[0])
    q = (t1[0] - t3[1], t1[1] + t3[0])
    return (o0, p, o2, q) if sgn < 0 else (o0, q, o2, p)


def _tw(x, e, sgn):
    r, i = x
    if e == 0:
        return x
    if e == 4:
        return (i, -r) if sgn < 0 else (-i, r)
    if e == 2:
        return ((r + i) * _R2, (i - r) * _R2) if sgn < 0 else ((r - i) * _R2, (r + i) * _R2)
    if e == 6:
        return ((i - r) * _R2, (r + i) * -_R2) if sgn < 0 else ((r + i) * -_R2, (r - i) * _R2)
    c = float(np.cos(2 * np.pi * e / 16))
    s = sgn * float(np.sin(2 * np.pi * e / 16))
    return (r * c - i * s, r * s + i * c)


_TWC = (16, 32, 24, 32)


def _lo(w):
    return pltpu.bitcast(w << 16, f32)


def _hi(w):
    return pltpu.bitcast(w & u32(0xFFFF0000), f32)


def _pack(a, b):
    return pltpu.pack_elementwise([a, b], packed_dtype=bf16).astype(u32)


def _gelu(h):
    c1 = 0.7978845608028654
    u = h * (c1 + (c1 * 0.044715) * (h * h))
    hh = 0.5 * h
    return hh + hh * jnp.tanh(u)


class _Fill:
    def __init__(self, steps):
        self.it = iter(steps)
        self.debt = 0

    def __call__(self, budget):
        self.debt += budget
        while self.debt > 0:
            c = next(self.it, None)
            if c is None:
                return
            self.debt -= c


def _kernel(q_hbm, k_hbm, v_hbm, sk_ref, ssm_hbm, d_ref, w1_hbm, b1_ref, w2_hbm, b2_ref,
            fwd_hbm, inv_hbm, o_hbm,
            q_buf, k_buf, v_buf, ssm_buf, w1_buf, w2_buf, fwd_buf, inv_buf,
            kt_buf, rhs_buf, ya, yb, z_buf, y_buf, xn_buf, acc, o_buf, b1_buf, b2_buf, sems, osems):
    cps = {}

    def start(name, src, dst):
        cp = pltpu.make_async_copy(src, dst, sems.at[len(cps)])
        cp.start()
        cps[name] = cp

    qw, kw, vw, sw = (r.bitcast(u32) for r in (q_hbm, k_hbm, v_hbm, ssm_hbm))
    HB = BM // 2
    start("q0", qw.at[0, pl.ds(0, HB)], q_buf.at[pl.ds(0, HB)])
    w1w, w2w = w1_hbm.bitcast(u32), w2_hbm.bitcast(u32)
    for f0 in range(0, F, WC):
        rs = pl.ds(f0 // 2, (min(F, f0 + WC) - f0) // 2)
        start(("w1", f0), w1w.at[rs], w1_buf.at[rs])

    def mlp(i, side=(), first=False):
        r = pl.ds(pl.multiple_of(i * BM, BM), BM)
        rw = pl.ds(pl.multiple_of(i * HB, HB), HB)
        x = pltpu.bitcast(q_buf[rw, :], bf16).astype(f32)
        m = jnp.mean(x, axis=-1, keepdims=True)
        xc = x - m
        var = jnp.mean(xc * xc, axis=-1, keepdims=True)
        xn = (xc * jax.lax.rsqrt(var + 1e-5)).astype(bf16)
        for g in range(G):
            xn_buf[g, r, :] = xn[:, g * 128:(g + 1) * 128]
        fill = _Fill(side)
        hs = []
        for j, f0 in enumerate(range(0, F, 128)):
            f1 = min(F, f0 + 128)
            if first and f0 % WC == 0:
                cps["w1", f0].wait()
                g = f0 // WC
                if g < G:
                    ls = pl.ds(g * 128, 128)
                    start(("w2", g), w2w.at[:, ls], w2_buf.at[:, ls])
            h = jax.lax.dot_general(xn, pltpu.bitcast(w1_buf[f0 // 2:f1 // 2, :], bf16),
                                    (((1,), (1,)), ((), ())), preferred_element_type=f32)
            hs.append(_gelu(h + b1_buf[:, f0:f1]).astype(bf16))
            fill(FILL1)
        KH = 512
        for g in range(G):
            ls = slice(g * 128, (g + 1) * 128)
            if first:
                cps["w2", g].wait()
                if g == 0:
                    start("q1", qw.at[0, pl.ds(HB, S // 2 - HB)], q_buf.at[pl.ds(HB, S // 2 - HB)])
            o = x[:, ls] + b2_buf[:, ls]
            for f0 in range(0, F, KH):
                f1 = min(F, f0 + KH)
                h = jnp.concatenate(hs[f0 // 128:(f1 + 127) // 128], axis=1)
                o = o + jnp.dot(h, pltpu.bitcast(w2_buf[f0 // 2:f1 // 2, ls], bf16),
                                preferred_element_type=f32)
                fill(FILL2 * (f1 - f0) // 128)
            acc[g, r, :] = o
        fill(10**9)

    def prep(g):
        sk = sk_ref[g].astype(f32)
        sk = [jnp.broadcast_to(sk[j:j + 1, :], (8, 128)) for j in range(KS)]
        rs = pl.ds(pl.multiple_of(g * 64, 64), 64)
        for a in range(8):
            lo, hi = (pltpu.bitcast(ssm_buf[rs, c:c + 128], bf16).astype(f32)
                      for c in (128 * a, 128 * a + S // 2))
            kt = _pack(lo, hi).T
            for j in range(8):
                kt_buf[g, pl.ds(KP * (8 * a + j), N2), :] = kt[N2 * j:N2 * (j + 1)]
            yield 64
            res = []
            for hf in range(2):
                base = a * 64 + hf * 512
                w = [kw_ld(g, base + 8 + m) for m in range(-2, 8)]
                ks = [f(x) for x in w for f in (_lo, _hi)]
                kv = []
                for m in range(8):
                    w = v_buf[g, pl.ds(base + m, 8, stride=8), :]
                    for p, vv in enumerate((_lo(w), _hi(w))):
                        n = 4 + 2 * m + p
                        s = (ks[n] * sk[0] + ks[n - 1] * sk[1]) + (ks[n - 2] * sk[2] + ks[n - 3] * sk[3])
                        kv.append(s * vv)
                res.append(kv)
                yield 172
            for n in range(N2):
                rhs_buf[g, n, pl.ds(a * 8, 8), :] = _pack(res[0][n], res[1][n])

    def kw_ld(g, r):
        return k_buf[g, pl.ds(r, 8, stride=8), :]

    def stage1(g, side=()):
        fill = _Fill(side)
        dd = d_ref[g].astype(f32)
        row = jax.lax.broadcasted_iota(jnp.int32, (8, 128), 0)
        dd = jnp.where(row == 0, jnp.broadcast_to(dd, (8, 128)), 0.0)
        for n in range(N2):
            kk = kt_buf[g, pl.ds(n, N1 // 2, stride=KP), :]
            if n == 0:
                top = _pack(_lo(kk[:8]) + dd, _hi(kk[:8]))
                kk = jnp.concatenate([top, kk[8:]], axis=0)
            rhs = pltpu.bitcast(jnp.concatenate([rhs_buf[g, n], kk], axis=1), bf16)
            y = jnp.dot(pltpu.bitcast(fwd_buf[n], bf16), rhs, preferred_element_type=f32)
            ya[g, n] = y[:, 0:128]
            yb[g, n] = y[:, 128:256]
            fill(210)
        fill(10**9)

    def middle(g):
        for a in range(0, N1, 8):
            ys = []
            for ref in (yb, ya):
                y = [[None] * 4 for _ in range(4)]
                for b in range(4):
                    x = [(ref[g, n, pl.ds(a, 8), :], ref[g, n, pl.ds(N1 + a, 8), :])
                         for n in range(b, N2, 4)]
                    o = _bf4(*x, -1)
                    for c in range(4):
                        y[c][b] = _tw(o[c], b * c, -1)
                    yield _TWC[b]
                ys.append(y)
            w = [[None] * 4 for _ in range(4)]
            for c in range(4):
                fb = _bf4(*ys[0][c], -1)
                fa = _bf4(*ys[1][c], -1)
                pr = [(p[0] * q[0] - p[1] * q[1], p[0] * q[1] + p[1] * q[0]) for p, q in zip(fa, fb)]
                o = _bf4(*pr, 1)
                for e in range(4):
                    w[e][c] = _tw(o[e], c * e, 1)
                yield 56 + _TWC[c]
            for e in range(4):
                o = _bf4(*w[e], 1)
                for d in range(4):
                    z_buf[g, e + 4 * d, pl.ds(a, 8), :] = _pack(*o[d])
                yield 20

    def inverse(g, side=()):
        fill = _Fill(side)
        for m in range(N2 // 2):
            y0, y1 = (jnp.dot(pltpu.bitcast(inv_buf[n], bf16), pltpu.bitcast(z_buf[g, n], bf16),
                              preferred_element_type=f32) for n in (2 * m, 2 * m + 1))
            y_buf[g, pl.ds(m, N1, stride=8), :] = _pack(y0, y1)
            fill(1)

    def out_copy(g):
        return pltpu.make_async_copy(
            o_buf.at[g], o_hbm.at[0, :, pl.ds(pl.multiple_of(g * 128, 128), 128)],
            osems.at[g])

    def final(g):
        for i in range(NB):
            r = pl.ds(i * BM, BM)
            y = pltpu.bitcast(y_buf[g, pl.ds(i * HB, HB), :], bf16).astype(f32)
            o_buf[g, r, :] = (acc[g, r, :] + xn_buf[g, r, :].astype(f32) * y).astype(bf16)
            yield 1
        out_copy(g).start()

    for g in range(G):
        k_buf[g, pl.ds(0, 8), :] = jnp.zeros((8, 128), u32)
    b1_buf[...] = b1_ref[...].astype(f32).reshape(1, F)
    b2_buf[...] = b2_ref[...].astype(f32).reshape(1, D)
    cps["q0"].wait()
    mlp(0, first=True)
    start("ssm", sw, ssm_buf)
    for g in range(G):
        ls = pl.ds(g * 128, 128)
        start(("k", g), kw.at[0, :, ls], k_buf.at[g, pl.ds(8, S // 2)])
        start(("v", g), vw.at[0, :, ls], v_buf.at[g])
    start("fwd", fwd_hbm, fwd_buf)
    start("inv", inv_hbm, inv_buf)
    cps["q1"].wait()

    pl.loop(1, NB - G)(mlp)
    for n in cps:
        if n[0] not in ("q", "w1", "w2"):
            cps[n].wait()
    _Fill(prep(0))(10**9)

    @pl.loop(0, G - 1)
    def _(g):
        stage1(g, prep(g + 1))

    stage1(G - 1)

    @pl.loop(0, G)
    def _(g):
        mlp(g + (NB - G), middle(g))

    inverse(0)

    @pl.loop(1, G)
    def _(g):
        side = final(g - 1)
        inverse(g, side)
        _Fill(side)(10**9)

    _Fill(final(G - 1))(10**9)
    for g in range(G):
        out_copy(g).wait()


FILL1, FILL2 = 220, 100
WC = 256
KP = 24


def _words(m):
    u = np.ascontiguousarray(m).view(np.uint16).astype(np.uint32)
    return u[..., 0::2, :] | (u[..., 1::2, :] << 16)


def _perm_fwd():
    r = np.arange(N1)
    n1 = r // 2 + (N1 // 2) * (r % 2)
    return _words(_FWD[:, :, n1])


_FWD_P = _perm_fwd()
_INV_P = _words(_INV)


@jax.jit
def pallas_parallel_sum__ssm_conv_h3__dense_activation_gelu__prompt_kernel(
    A_q, A_k, A_v, A_shift_k, A_ssm_k, A_ssm_D, B_x, B_w1, B_b1, B_w2, B_b2,
):
    hbm = pl.BlockSpec(memory_space=pl.ANY)
    vmem = pl.BlockSpec(memory_space=pltpu.VMEM)
    return pl.pallas_call(
        _kernel,
        out_shape=jax.ShapeDtypeStruct((1, S, D), bf16),
        in_specs=[hbm, hbm, hbm, vmem, hbm, vmem, hbm, vmem, hbm, vmem, hbm, hbm],
        out_specs=hbm,
        scratch_shapes=[
            pltpu.VMEM((S // 2, D), u32),
            pltpu.VMEM((G, S // 2 + 8, 128), u32),
            pltpu.VMEM((G, S // 2, 128), u32),
            pltpu.VMEM((D // 2, S), u32),
            pltpu.VMEM((F // 2, D), u32),
            pltpu.VMEM((F // 2, D), u32),
            pltpu.VMEM((N2, N1, N1), u32),
            pltpu.VMEM((N2, N1 // 2, 2 * N1), u32),
            pltpu.VMEM((G, KP * N1 // 2, 128), u32),
            pltpu.VMEM((G, N2, N1 // 2, 128), u32),
            pltpu.VMEM((G, N2, 2 * N1, 128), f32),
            pltpu.VMEM((G, N2, 2 * N1, 128), f32),
            pltpu.VMEM((G, N2, N1, 128), u32),
            pltpu.VMEM((G, S // 2, 128), u32),
            pltpu.VMEM((G, S, 128), bf16),
            pltpu.VMEM((G, S, 128), f32),
            pltpu.VMEM((G, S, 128), bf16),
            pltpu.VMEM((1, F), f32),
            pltpu.VMEM((1, D), f32),
            pltpu.SemaphoreType.DMA((27,)),
            pltpu.SemaphoreType.DMA((G,)),
        ],
        compiler_params=pltpu.CompilerParams(vmem_limit_bytes=100 * 2**20),
    )(A_q, A_k, A_v, A_shift_k.T.reshape(KS, G, 128).transpose(1, 0, 2), A_ssm_k,
      A_ssm_D.reshape(G, 1, 128), B_w1.T, B_b1, B_w2, B_b2, _FWD_P, _INV_P)
```

```python
import contextlib

import jax
import jax.numpy as jnp
import numpy as np
import jax.experimental.pallas as pl
import jax.experimental.pallas.tpu as pltpu

S, D, F, KS = 2048, 640, 1728, 4
N1, N2 = 128, 16
G = D // 128
BM = 256
NB = S // BM
bf16, f32, u32 = jnp.bfloat16, jnp.float32, jnp.uint32


def _dft_mats():
    k1 = np.arange(N1)[None, :, None]
    n1 = np.arange(N1)[None, None, :]
    n2 = np.arange(N2)[:, None, None]
    ang = -2.0 * np.pi * (k1 + 0.25) * (N2 * n1 + n2) / S
    fr, fi = np.cos(ang), np.sin(ang)
    fwd = np.concatenate([fr, fi], axis=1)
    inv = np.stack([fr, fi], axis=2).reshape(N2, 2 * N1, N1)
    inv = np.transpose(inv, (0, 2, 1)) / S
    return fwd.astype(jnp.bfloat16), inv.astype(jnp.bfloat16)


_FWD, _INV = _dft_mats()

_C1, _S1, _R2 = float(np.cos(np.pi / 8)), float(np.sin(np.pi / 8)), float(np.sqrt(0.5))


def _bf4(a, b, c, d, sgn):
    t0 = (a[0] + c[0], a[1] + c[1])
    t1 = (a[0] - c[0], a[1] - c[1])
    t2 = (b[0] + d[0], b[1] + d[1])
    t3 = (b[0] - d[0], b[1] - d[1])
    o0 = (t0[0] + t2[0], t0[1] + t2[1])
    o2 = (t0[0] - t2[0], t0[1] - t2[1])
    p = (t1[0] + t3[1], t1[1] - t3[0])
    q = (t1[0] - t3[1], t1[1] + t3[0])
    return (o0, p, o2, q) if sgn < 0 else (o0, q, o2, p)


def _tw(x, e, sgn):
    r, i = x
    if e == 0:
        return x
    if e == 4:
        return (i, -r) if sgn < 0 else (-i, r)
    if e == 2:
        return ((r + i) * _R2, (i - r) * _R2) if sgn < 0 else ((r - i) * _R2, (r + i) * _R2)
    if e == 6:
        return ((i - r) * _R2, (r + i) * -_R2) if sgn < 0 else ((r + i) * -_R2, (r - i) * _R2)
    c = float(np.cos(2 * np.pi * e / 16))
    s = sgn * float(np.sin(2 * np.pi * e / 16))
    return (r * c - i * s, r * s + i * c)


_TWC = (16, 32, 24, 32)


def _lo(w):
    return pltpu.bitcast(w << 16, f32)


def _hi(w):
    return pltpu.bitcast(w & u32(0xFFFF0000), f32)


def _pack(a, b):
    return pltpu.pack_elementwise([a, b], packed_dtype=bf16).astype(u32)


def _gelu(h):
    c1 = 0.7978845608028654
    u = h * (c1 + (c1 * 0.044715) * (h * h))
    hh = 0.5 * h
    return hh + hh * jnp.tanh(u)


def _scope(name):
    return contextlib.nullcontext()


class _Fill:
    def __init__(self, steps):
        self.it = iter(steps)
        self.debt = 0

    def __call__(self, budget):
        self.debt += budget
        while self.debt > 0:
            c = next(self.it, None)
            if c is None:
                return
            self.debt -= c


def _kernel(q_hbm, k_hbm, v_hbm, sk_ref, ssm_hbm, d_ref, w1_hbm, b1_ref, w2_hbm, b2_ref,
            fwd_hbm, inv_hbm, o_hbm,
            q_buf, k_buf, v_buf, ssm_buf, w1_buf, w2_buf, fwd_buf, inv_buf,
            kt_buf, rhs_buf, ya, yb, z_buf, y_buf, xn_buf, h_buf, acc, o_buf, b1_buf, b2_buf, sems, osems):
    cps = {}

    def start(name, src, dst):
        cp = pltpu.make_async_copy(src, dst, sems.at[len(cps)])
        cp.start()
        cps[name] = cp

    qw, kw, vw, sw = (r.bitcast(u32) for r in (q_hbm, k_hbm, v_hbm, ssm_hbm))
    HB = BM // 2
    w1w, w2w = w1_hbm.bitcast(u32), w2_hbm.bitcast(u32)

    def start_q(b0, b1):
        rs = pl.ds(b0 * HB, (b1 - b0) * HB)
        start(("q", b0), qw.at[0, rs], q_buf.at[rs])

    def start_w1(c):
        rs = pl.ds(WCH[c] // 2, (WCH[c + 1] - WCH[c]) // 2)
        start(("w1", WCH[c]), w1w.at[rs], w1_buf.at[rs])

    def rows(i, n):
        return pl.ds(i * n if isinstance(i, int) else pl.multiple_of(i * n, n), n)

    def norm(*blocks):
        for i in blocks:
            for c in range(BM // LC):
                x = pltpu.bitcast(q_buf[rows(i * (BM // LC) + c, LC // 2), :], bf16).astype(f32)
                m = jnp.mean(x, axis=-1, keepdims=True)
                xc = x - m
                var = jnp.mean(xc * xc, axis=-1, keepdims=True)
                xn = (xc * jax.lax.rsqrt(var + 1e-5)).astype(bf16)
                xn_buf[rows(i * (BM // LC) + c, LC // 2), :] = pltpu.bitcast(xn, u32)
                yield LC * 6

    def mm1(i, fill, cost, before=lambda f0: None):
        for j, f0 in enumerate(range(0, F, 128)):
            f1 = min(F, f0 + 128)
            before(f0)
            xn = pltpu.bitcast(xn_buf[rows(i, HB), :], bf16)
            h = jax.lax.dot_general(xn, pltpu.bitcast(w1_buf[f0 // 2:f1 // 2, :], bf16),
                                    (((1,), (1,)), ((), ())), preferred_element_type=f32)
            h_buf[rows(i, HB), f0:f1] = pltpu.bitcast(_gelu(h + b1_buf[:, f0:f1]).astype(bf16), u32)
            fill(cost)

    def mm2(i, fill, cost):
        for g in range(G):
            ls = slice(g * 128, (g + 1) * 128)
            o = pltpu.bitcast(q_buf[rows(i, HB), ls], bf16).astype(f32) + b2_buf[:, ls]
            for f0 in range(0, F, KH):
                f1 = min(F, f0 + KH)
                h = pltpu.bitcast(h_buf[rows(i, HB), f0:f1], bf16)
                o = o + jnp.dot(h, pltpu.bitcast(w2_buf[f0 // 2:f1 // 2, ls], bf16),
                                preferred_element_type=f32)
                fill(cost * (f1 - f0) // 128)
            acc[g, rows(i, BM), :] = o

    def prep(g):
        sk = sk_ref[:, g * 128:(g + 1) * 128].astype(f32)
        sk = [jnp.broadcast_to(sk[j:j + 1, :], (8, 128)) for j in range(KS)]
        rs = rows(g, 64)
        for a in range(8):
            lo, hi = (pltpu.bitcast(ssm_buf[rs, c:c + 128], bf16).astype(f32)
                      for c in (128 * a, 128 * a + S // 2))
            kt = _pack(lo, hi).T
            for j in range(8):
                kt_buf[g, pl.ds(KP * (8 * a + j), N2), :] = kt[N2 * j:N2 * (j + 1)]
            yield 96
            res = []
            for hf in range(2):
                base = a * 64 + hf * 512
                w = [kw_ld(g, base + 8 + m) for m in range(-2, 8)]
                ks = [f(x) for x in w for f in (_lo, _hi)]
                kv = []
                for m in range(8):
                    w = v_buf[g, pl.ds(base + m, 8, stride=8), :]
                    for p, vv in enumerate((_lo(w), _hi(w))):
                        n = 4 + 2 * m + p
                        s = (ks[n] * sk[0] + ks[n - 1] * sk[1]) + (ks[n - 2] * sk[2] + ks[n - 3] * sk[3])
                        kv.append(s * vv)
                res.append(kv)
                yield 172
            for n in range(N2):
                rhs_buf[g, n, pl.ds(a * 8, 8), :] = _pack(res[0][n], res[1][n])

    def kw_ld(g, r):
        return k_buf[g, pl.ds(r, 8, stride=8), :]

    def stage1(g, side=()):
        fill = _Fill(side)
        dd = d_ref[...].astype(f32).reshape(1, D)[:, g * 128:(g + 1) * 128]
        row = jax.lax.broadcasted_iota(jnp.int32, (8, 128), 0)
        dd = jnp.where(row == 0, jnp.broadcast_to(dd, (8, 128)), 0.0)
        for n in range(N2):
            kk = kt_buf[g, pl.ds(n, N1 // 2, stride=KP), :]
            if n == 0:
                top = _pack(_lo(kk[:8]) + dd, _hi(kk[:8]))
                kk = jnp.concatenate([top, kk[8:]], axis=0)
            rhs = pltpu.bitcast(jnp.concatenate([rhs_buf[g, n], kk], axis=1), bf16)
            y = jnp.dot(pltpu.bitcast(fwd_buf[n], bf16), rhs, preferred_element_type=f32)
            ya[g, n] = y[:, 0:128]
            yb[g, n] = y[:, 128:256]
            fill(225)
        fill(ALL)

    def middle(g):
        for a in range(0, N1, 8):
            ys = []
            for ref in (yb, ya):
                y = [[None] * 4 for _ in range(4)]
                for b in range(4):
                    x = [(ref[g, n, pl.ds(a, 8), :], ref[g, n, pl.ds(N1 + a, 8), :])
                         for n in range(b, N2, 4)]
                    o = _bf4(*x, -1)
                    for c in range(4):
                        y[c][b] = _tw(o[c], b * c, -1)
                    yield _TWC[b]
                ys.append(y)
            w = [[None] * 4 for _ in range(4)]
            for c in range(4):
                fb = _bf4(*ys[0][c], -1)
                fa = _bf4(*ys[1][c], -1)
                pr = [(p[0] * q[0] - p[1] * q[1], p[0] * q[1] + p[1] * q[0]) for p, q in zip(fa, fb)]
                o = _bf4(*pr, 1)
                for e in range(4):
                    w[e][c] = _tw(o[e], c * e, 1)
                yield 56 + _TWC[c]
            for e in range(4):
                o = _bf4(*w[e], 1)
                for d in range(4):
                    z_buf[g, e + 4 * d, pl.ds(a, 8), :] = _pack(*o[d])
                yield 20

    def inverse(g, side=()):
        fill = _Fill(side)
        for m in range(N2 // 2):
            y0, y1 = (jnp.dot(pltpu.bitcast(inv_buf[n], bf16), pltpu.bitcast(z_buf[g, n], bf16),
                              preferred_element_type=f32) for n in (2 * m, 2 * m + 1))
            y_buf[g, pl.ds(m, N1, stride=8), :] = _pack(y0, y1)
            fill(1)

    def out_copy(g):
        return pltpu.make_async_copy(
            o_buf.at[g], o_hbm.at[0, :, rows(g, 128)],
            osems.at[g])

    def final(g):
        for i in range(NB):
            r = pl.ds(i * BM, BM)
            y = pltpu.bitcast(y_buf[g, pl.ds(i * HB, HB), :], bf16).astype(f32)
            xn = pltpu.bitcast(xn_buf[pl.ds(i * HB, HB), rows(g, 128)], bf16)
            o_buf[g, r, :] = (acc[g, r, :] + xn.astype(f32) * y).astype(bf16)
            yield 1
        out_copy(g).start()

    start_q(0, 1)
    start_w1(0)
    start_w1(1)
    for g in range(G):
        k_buf[g, pl.ds(0, 8), :] = jnp.zeros((8, 128), u32)
    b1_buf[...] = b1_ref[...].astype(f32).reshape(1, F)
    b2_buf[...] = b2_ref[...].astype(f32).reshape(1, D)
    def w1_ready(f0):
        if f0 in WCH:
            cps["w1", f0].wait()
            if f0 == WCH[0]:
                start_w1(2)
                start_q(1, 4)
            if f0 == WCH[1]:
                start("w2", w2w, w2_buf)
                start_q(4, NB)

    with _scope("M0"):
        cps["q", 0].wait()
        _Fill(norm(0))(ALL)
        mm1(0, _Fill(()), 0, w1_ready)
        start("ssm", sw, ssm_buf)
        start("fwd", fwd_hbm, fwd_buf)
        cps["q", 1].wait()
        _Fill(norm(1))(ALL)
        fill = _Fill(norm(2, 3))
        mm1(1, fill, 250)
        fill(ALL)
        for g in range(G):
            ls = pl.ds(g * 128, 128)
            start(("k", g), kw.at[0, :, ls], k_buf.at[g, pl.ds(8, S // 2)])
            start(("v", g), vw.at[0, :, ls], v_buf.at[g])
        cps["w2"].wait()
        cps["q", 4].wait()

    with _scope("A"):
        @pl.loop(0, 2)
        def _(i):
            fill = _Fill(norm(4 + 2 * i, 5 + 2 * i))
            mm2(i, fill, 80)
            fill(ALL)
            mm1(i + 2, fill, 0)

    for n in cps:
        if n[0] not in ("q", "w1") and n != "w2":
            cps[n].wait()
    start("inv", inv_hbm, inv_buf)
    with _scope("prep0"):
        _Fill(prep(0))(ALL)
    with _scope("B"):
        for g in range(G - 1):
            stage1(g, prep(g + 1))

    with _scope("S4"):
        stage1(G - 1)

    with _scope("C"):
        @pl.loop(0, G - 1)
        def _(g):
            fill = _Fill(middle(g))
            mm2(g + 2, fill, FILL2)
            mm1(g + 4, fill, FILL1)
            fill(ALL)

    with _scope("E"):
        fill = _Fill(middle(G - 1))
        mm2(NB - 2, fill, 75)
        mm2(NB - 1, fill, 75)
        fill(ALL)

    cps["inv"].wait()
    with _scope("I0"):
        inverse(0)

    with _scope("Dd"):
        for g in range(1, G):
            side = final(g - 1)
            inverse(g, side)
            _Fill(side)(ALL)

    with _scope("F4"):
        _Fill(final(G - 1))(ALL)
    for g in range(G):
        out_copy(g).wait()


FILL1, FILL2 = 220, 100
ALL = 10**9
WCH = (0, 512, 1024, F)
NF = (F + 127) // 128
KH = 512
LC = 64
KP = 24


def _words(m):
    u = np.ascontiguousarray(m).view(np.uint16).astype(np.uint32)
    return u[..., 0::2, :] | (u[..., 1::2, :] << 16)


def _perm_fwd():
    r = np.arange(N1)
    n1 = r // 2 + (N1 // 2) * (r % 2)
    return _words(_FWD[:, :, n1])


_FWD_P = _perm_fwd()
_INV_P = _words(_INV)


@jax.jit
def pallas_parallel_sum__ssm_conv_h3__dense_activation_gelu__prompt_kernel(
    A_q, A_k, A_v, A_shift_k, A_ssm_k, A_ssm_D, B_x, B_w1, B_b1, B_w2, B_b2,
):
    hbm = pl.BlockSpec(memory_space=pl.ANY)
    vmem = pl.BlockSpec(memory_space=pltpu.VMEM)
    return pl.pallas_call(
        _kernel,
        out_shape=jax.ShapeDtypeStruct((1, S, D), bf16),
        in_specs=[hbm, hbm, hbm, vmem, hbm, vmem, hbm, vmem, hbm, vmem, hbm, hbm],
        out_specs=hbm,
        scratch_shapes=[
            pltpu.VMEM((S // 2, D), u32),
            pltpu.VMEM((G, S // 2 + 8, 128), u32),
            pltpu.VMEM((G, S // 2, 128), u32),
            pltpu.VMEM((D // 2, S), u32),
            pltpu.VMEM((F // 2, D), u32),
            pltpu.VMEM((F // 2, D), u32),
            pltpu.VMEM((N2, N1, N1), u32),
            pltpu.VMEM((N2, N1 // 2, 2 * N1), u32),
            pltpu.VMEM((G, KP * N1 // 2, 128), u32),
            pltpu.VMEM((G, N2, N1 // 2, 128), u32),
            pltpu.VMEM((G, N2, 2 * N1, 128), f32),
            pltpu.VMEM((G, N2, 2 * N1, 128), f32),
            pltpu.VMEM((G, N2, N1, 128), u32),
            pltpu.VMEM((G, S // 2, 128), u32),
            pltpu.VMEM((S // 2, D), u32),
            pltpu.VMEM((S // 2, F), u32),
            pltpu.VMEM((G, S, 128), f32),
            pltpu.VMEM((G, S, 128), bf16),
            pltpu.VMEM((1, F), f32),
            pltpu.VMEM((1, D), f32),
            pltpu.SemaphoreType.DMA((19,)),
            pltpu.SemaphoreType.DMA((G,)),
        ],
        compiler_params=pltpu.CompilerParams(vmem_limit_bytes=100 * 2**20),
    )(A_q, A_k, A_v, A_shift_k.T, A_ssm_k,
      A_ssm_D, B_w1.T, B_b1, B_w2, B_b2, _FWD_P, _INV_P)
```

```python
import contextlib

import jax
import jax.numpy as jnp
import numpy as np
import jax.experimental.pallas as pl
import jax.experimental.pallas.tpu as pltpu

S, D, F, KS = 2048, 640, 1728, 4
N1, N2 = 128, 16
G = D // 128
BM = 256
NB = S // BM
bf16, f32, u32 = jnp.bfloat16, jnp.float32, jnp.uint32


def _dft_mats():
    k1 = np.arange(N1)[None, :, None]
    n1 = np.arange(N1)[None, None, :]
    n2 = np.arange(N2)[:, None, None]
    ang = -2.0 * np.pi * (k1 + 0.25) * (N2 * n1 + n2) / S
    fr, fi = np.cos(ang), np.sin(ang)
    fwd = np.concatenate([fr, fi], axis=1)
    inv = np.stack([fr, fi], axis=2).reshape(N2, 2 * N1, N1)
    inv = np.transpose(inv, (0, 2, 1)) / S
    return fwd.astype(jnp.bfloat16), inv.astype(jnp.bfloat16)


_FWD, _INV = _dft_mats()

_C1, _S1, _R2 = float(np.cos(np.pi / 8)), float(np.sin(np.pi / 8)), float(np.sqrt(0.5))


def _bf4(a, b, c, d, sgn):
    t0 = (a[0] + c[0], a[1] + c[1])
    t1 = (a[0] - c[0], a[1] - c[1])
    t2 = (b[0] + d[0], b[1] + d[1])
    t3 = (b[0] - d[0], b[1] - d[1])
    o0 = (t0[0] + t2[0], t0[1] + t2[1])
    o2 = (t0[0] - t2[0], t0[1] - t2[1])
    p = (t1[0] + t3[1], t1[1] - t3[0])
    q = (t1[0] - t3[1], t1[1] + t3[0])
    return (o0, p, o2, q) if sgn < 0 else (o0, q, o2, p)


def _tw(x, e, sgn):
    r, i = x
    if e == 0:
        return x
    if e == 4:
        return (i, -r) if sgn < 0 else (-i, r)
    if e == 2:
        return ((r + i) * _R2, (i - r) * _R2) if sgn < 0 else ((r - i) * _R2, (r + i) * _R2)
    if e == 6:
        return ((i - r) * _R2, (r + i) * -_R2) if sgn < 0 else ((r + i) * -_R2, (r - i) * _R2)
    c = float(np.cos(2 * np.pi * e / 16))
    s = sgn * float(np.sin(2 * np.pi * e / 16))
    return (r * c - i * s, r * s + i * c)


_TWC = (16, 32, 24, 32)


def _lo(w):
    return pltpu.bitcast(w << 16, f32)


def _hi(w):
    return pltpu.bitcast(w & u32(0xFFFF0000), f32)


def _pack(a, b):
    return pltpu.pack_elementwise([a, b], packed_dtype=bf16).astype(u32)


def _gelu(h):
    c1 = 0.7978845608028654
    u = h * (c1 + (c1 * 0.044715) * (h * h))
    if not FOLD:
        h = 0.5 * h
    return h + h * jnp.tanh(u)


def _scope(name):
    return contextlib.nullcontext()


class _Fill:
    def __init__(self, steps):
        self.it = iter(steps)
        self.debt = 0

    def __call__(self, budget):
        self.debt += budget
        while self.debt > 0:
            c = next(self.it, None)
            if c is None:
                return
            self.debt -= c


def _kernel(q_hbm, k_hbm, v_hbm, sk_ref, ssm_hbm, d_ref, w1_hbm, b1_ref, w2_hbm, b2_ref,
            fwd_hbm, inv_hbm, zero_ref, o_hbm,
            q_buf, k_buf, v_buf, ssm_buf, w1_buf, w2_buf, fwd_buf, inv_buf,
            kt_buf, rhs_buf, y_buf, xn_buf, h_buf, acc, fb, b1_buf, b2_buf, sems, osems):
    qw, kw, vw, sw, w1w, w2w = (r.bitcast(u32) for r in (q_hbm, k_hbm, v_hbm, ssm_hbm, w1_hbm, w2_hbm))
    HB = BM // 2
    ya, yb = 0, 1
    z0 = zero_ref[0]

    def copy(name):
        kind, i = name
        if kind == "q":
            rs = pl.ds(QCH[i] * HB, (QCH[i + 1] - QCH[i]) * HB)
            src, dst = qw.at[0, rs], q_buf.at[rs]
        elif kind == "w1":
            rs = pl.ds(WCH[i] // 2, (WCH[i + 1] - WCH[i]) // 2)
            src, dst = w1w.at[rs], w1_buf.at[rs]
        elif kind == "ssm":
            src, dst = sw.at[rows(i, 64)], ssm_buf.at[rows(i, 64)]
        elif kind == "k":
            src, dst = kw.at[0, :, rows(i, 128)], k_buf.at[i, pl.ds(8, S // 2)]
        elif kind == "v":
            src, dst = vw.at[0, :, rows(i, 128)], v_buf.at[i]
        else:
            src, dst = ((w2w, w2_buf), (fwd_hbm, fwd_buf), (inv_hbm, inv_buf))[i]
        return pltpu.make_async_copy(src, dst, sems.at[COPIES.index(name)])

    def start(*names):
        for name in names:
            copy(name).start()

    def wait(*names):
        for name in names:
            copy(name).wait()

    def conv_in(*groups):
        return [(kind, g) for g in groups for kind in ("ssm", "k", "v")]

    def rows(i, n):
        return pl.ds(i * n if isinstance(i, int) else pl.multiple_of(i * n, n), n)

    def norm(*blocks, cost=LC * 6):
        for i in blocks:
            for c in range(BM // LC):
                x = pltpu.bitcast(q_buf[rows(i * (BM // LC) + c, LC // 2), :], bf16).astype(f32)
                m = jnp.mean(x, axis=-1, keepdims=True)
                xc = x - m
                var = jnp.mean(xc * xc, axis=-1, keepdims=True)
                xn = (xc * jax.lax.rsqrt(var + 1e-5)).astype(bf16)
                xn_buf[rows(i * (BM // LC) + c, LC // 2), :] = pltpu.bitcast(xn, u32)
                yield cost

    def mm1(i, fill, cost, lo=0, hi=F):
        for f0 in range(lo, hi, 128):
            f1 = min(F, f0 + 128)
            xn = pltpu.bitcast(xn_buf[rows(i, HB), :], bf16)
            h = jax.lax.dot_general(xn, pltpu.bitcast(w1_buf[f0 // 2:f1 // 2, :], bf16),
                                    (((1,), (1,)), ((), ())), preferred_element_type=f32)
            h_buf[rows(i, HB), f0:f1] = pltpu.bitcast(_gelu(h + b1_buf[:, f0:f1]).astype(bf16), u32)
            fill(cost)

    def mm2(i, fill, cost, last=False, omem=False, gs=range(G)):
        for g in gs:
            ls = slice(g * 128, (g + 1) * 128)
            for f0 in range(0, F, KH):
                f1 = min(F, f0 + KH)
                h = pltpu.bitcast(h_buf[rows(i, HB), f0:f1], bf16)
                if f0 == 0:
                    o = 0.0
                elif omem:
                    o = acc[g, rows(i + z0, BM), :]
                p = jnp.dot(h, pltpu.bitcast(w2_buf[f0 // 2:f1 // 2, ls], bf16),
                            preferred_element_type=f32)
                o = p if f0 == 0 else o + p
                if omem:
                    c = f0 // KH
                    x = pltpu.bitcast(q_buf[rows(4 * (i + z0) + c, HB // 4), ls], bf16).astype(f32)
                    o = [o[r:r + BM // 4] for r in range(0, BM, BM // 4)]
                    o[c] = o[c] + ((2.0 * (x + b2_buf[:, ls])) if FOLD else (x + b2_buf[:, ls]))
                    o = jnp.concatenate(o, axis=0)
                    if f1 == F and FOLD:
                        o = 0.5 * o
                elif (f1 == F if FOLD else f0 == 0):
                    x = pltpu.bitcast(q_buf[rows(i, HB), ls], bf16).astype(f32)
                    o = (0.5 * o if FOLD else o) + (x + b2_buf[:, ls])
                if last and f1 == F:
                    gate(i, g, o)
                elif omem or f1 == F:
                    acc[g, rows(i, BM), :] = o
                fill(cost * (f1 - f0) // 128)

    def prep(g):
        sk = sk_ref[:, g * 128:(g + 1) * 128].astype(f32)
        sk = [jnp.broadcast_to(sk[j:j + 1, :], (8, 128)) for j in range(KS)]
        rs = rows(g, 64)
        for a in range(8):
            lo, hi = (pltpu.bitcast(ssm_buf[rs, c:c + 128], bf16).astype(f32)
                      for c in (128 * a, 128 * a + S // 2))
            kt = _pack(lo, hi).T
            for j in range(8):
                kt_buf[g, pl.ds(KP * (8 * a + j), N2), :] = kt[N2 * j:N2 * (j + 1)]
            yield 96
            res = []
            for hf in range(2):
                base = a * 64 + hf * 512
                w = [kw_ld(g, base + 8 + m) for m in range(-2, 8)]
                ks = [f(x) for x in w for f in (_lo, _hi)]
                kv = []
                for m in range(8):
                    w = v_buf[g, pl.ds(base + m, 8, stride=8), :]
                    for p, vv in enumerate((_lo(w), _hi(w))):
                        n = 4 + 2 * m + p
                        s = (ks[n] * sk[0] + ks[n - 1] * sk[1]) + (ks[n - 2] * sk[2] + ks[n - 3] * sk[3])
                        kv.append(s * vv)
                res.append(kv)
                yield 172
            for n in range(N2):
                rhs_buf[g, n, pl.ds(a * 8, 8), :] = _pack(res[0][n], res[1][n])

    def kw_ld(g, r):
        return k_buf[g, pl.ds(r, 8, stride=8), :]

    def stage1(g, side=()):
        fill = _Fill(side)
        dd = d_ref[...].astype(f32).reshape(1, D)[:, g * 128:(g + 1) * 128]
        row = jax.lax.broadcasted_iota(jnp.int32, (8, 128), 0)
        dd = jnp.where(row == 0, jnp.broadcast_to(dd, (8, 128)), 0.0)
        for n in range(N2):
            kk = kt_buf[g, pl.ds(n, N1 // 2, stride=KP), :]
            if n == 0:
                top = _pack(_lo(kk[:8]) + dd, _hi(kk[:8]))
                kk = jnp.concatenate([top, kk[8:]], axis=0)
            rhs = pltpu.bitcast(jnp.concatenate([rhs_buf[g, n], kk], axis=1), bf16)
            y = jnp.dot(pltpu.bitcast(fwd_buf[n], bf16), rhs, preferred_element_type=f32)
            for src in range(2):
                for part in range(2):
                    fb[g, pl.ds(_yrow(src, n, part), N1), :] = (
                        y[part * N1:(part + 1) * N1, src * 128:(src + 1) * 128])
            fill(225)
        fill(ALL)

    def middle(u0, nu):
        for u in range(nu):
            g = (u0 + u) // (N1 // 8)
            a = pl.multiple_of((u0 + u) % (N1 // 8) * 8, 8)

            held = {}

            def ld(ref, ns):
                return [held.get((ref, n)) or
                        (fb[g, pl.ds(a + _yrow(ref, n, 0), 8), :], fb[g, pl.ds(a + _yrow(ref, n, 1), 8), :]) for n in ns]

            def st(ref, ns, vals):
                for n, (re, im) in zip(ns, vals):
                    if not (MIDMEM == 1 or (MIDMEM == 2 and ref == yb)):
                        held[ref, n] = (re, im)
                        continue
                    fb[g, pl.ds(a + _yrow(ref, n, 0), 8), :] = re
                    fb[g, pl.ds(a + _yrow(ref, n, 1), 8), :] = im

            for ref in (yb, ya):
                for b in range(4):
                    ns = range(b, N2, 4)
                    o = _bf4(*ld(ref, ns), -1)
                    st(ref, ns, [_tw(o[c], b * c, -1) for c in range(4)])
                    yield _TWC[b]
            for c in range(4):
                ns = range(4 * c, 4 * c + 4)
                sb = _bf4(*ld(yb, ns), -1)
                fa = _bf4(*ld(ya, ns), -1)
                pr = [(p[0] * q[0] - p[1] * q[1], p[0] * q[1] + p[1] * q[0]) for p, q in zip(fa, sb)]
                o = _bf4(*pr, 1)
                st(ya, ns, [_tw(o[e], c * e, 1) for e in range(4)])
                yield 56 + _TWC[c]
            for e in range(4):
                o = _bf4(*ld(ya, range(e, N2, 4)), 1)
                for d in range(4):
                    fb[g, pl.ds(a + (ZZ + (e + 4 * d) * N1), 8), :] = pltpu.bitcast(_pack(*o[d]), f32)
                yield 20

    def inverse(g):
        for m in range(N2 // 2):
            y0, y1 = (jnp.dot(pltpu.bitcast(inv_buf[n], bf16), pltpu.bitcast(fb[g, pl.ds(ZZ + n * N1, N1), :], bf16),
                              preferred_element_type=f32) for n in (2 * m, 2 * m + 1))
            y_buf[g, pl.ds(m, N1, stride=8), :] = _pack(y0, y1)

    def out_copy(j):
        rs = pl.ds(OCH[j] * HB, (OCH[j + 1] - OCH[j]) * HB)
        return pltpu.make_async_copy(q_buf.at[rs], o_hbm.bitcast(u32).at[0, rs], osems.at[j])

    def gate(i, g, o):
        y = pltpu.bitcast(y_buf[g, rows(i, HB), :], bf16).astype(f32)
        xn = pltpu.bitcast(xn_buf[rows(i, HB), rows(g, 128)], bf16).astype(f32)
        q_buf[rows(i, HB), rows(g, 128)] = pltpu.bitcast((o + xn * y).astype(bf16), u32)

    def final(blocks):
        for i in blocks:
            for g in range(G):
                gate(i, g, acc[g, rows(i, BM), :])
                yield 150

    start(("q", 0))
    start(("w1", 0))
    for g in range(G):
        k_buf[g, pl.ds(0, 8), :] = jnp.zeros((8, 128), u32)
    b1_buf[...] = b1_ref[...].astype(f32).reshape(1, F)
    b2_buf[...] = b2_ref[...].astype(f32).reshape(1, D)
    with _scope("M0"):
        wait(("q", 0))
        start(("q", 1))
        start(("w1", 1))
        _Fill(norm(0))(ALL)
        wait(("w1", 0))
        mm1(0, _Fill(()), 0, WCH[0], WCH[1])
        wait(("q", 1))
        start(("w1", 2))
        _Fill(norm(1))(ALL)
        mm1(1, _Fill(()), 0, WCH[0], WCH[1])
        wait(("w1", 1))
        start(("q", 2))
        start(W2)
        for i in range(2):
            mm1(i, _Fill(()), 0, WCH[1], WCH[2])
        wait(("w1", 2))
        wait(("q", 2))
        start(("q", 3))
        fill = _Fill(norm(2, 3))
        for i in range(2):
            mm1(i, fill, 250, WCH[2], WCH[3])
        fill(ALL)
        wait(W2)
        wait(("q", 3))
        start(FWD, *conv_in(0, 1, 2))

    with _scope("A"):
        @pl.loop(0, 2)
        def _(i):
            @pl.when(i == 1)
            def _():
                start(("q", 4), *conv_in(3, 4))

            fill = _Fill(norm(4 + i))
            mm2(i, fill, 40)
            fill(ALL)
            mm1(i + 2, fill, 0)

    wait(FWD, *conv_in(0, 1, 2))
    start(INV)
    with _scope("prep0"):
        _Fill(prep(0))(ALL)
    with _scope("B"):
        for g in range(G - 1):
            if g == 2:
                wait(("q", 4), *conv_in(3, 4))
            stage1(g, prep(g + 1))

    with _scope("S4"):
        stage1(G - 1, norm(6, 7, cost=450))

    with _scope("C"):
        @pl.loop(0, G - 1)
        def _(g):
            fill = _Fill(middle(g * NU, NU))
            if ORD == 0:
                mm2(g + 2, fill, FILL2, omem=OMEM)
                mm1(g + 4, fill, FILL1)
            elif ORD == 1:
                mm1(g + 4, fill, FILL1)
                mm2(g + 2, fill, FILL2, omem=OMEM)
            else:
                for t in range(G):
                    mm2(g + 2, fill, FILL2, omem=OMEM, gs=(t,))
                    mm1(g + 4, fill, FILL1, 384 * t, min(F, 384 * t + 384))
            fill(ALL)

    wait(INV)
    with _scope("I"):
        pl.loop(0, G)(inverse)

    with _scope("E"):
        fill = _Fill(final([i for i in range(NB - 2)]))
        mm2(NB - 2, fill, 70, last=True, omem=True)
        fill(ALL)

        out_copy(0).start()
        mm2(NB - 1, _Fill(()), 0, last=True)
        out_copy(1).start()
    out_copy(0).wait()
    out_copy(1).wait()


OCH = (0, NB - 1, NB)
FILL1, FILL2 = 340, 117
ALL = 10**9
WCH = (0, 256, 768, F)
QCH = (0, 1, 2, 4, 6, NB)
W2, FWD, INV = ("mat", 0), ("mat", 1), ("mat", 2)
COPIES = ([("q", i) for i in range(5)] + [("w1", i) for i in range(3)] + [W2, FWD, INV]
          + [(kind, g) for g in range(G) for kind in ("ssm", "k", "v")])
NU = G * (N1 // 8) // 4
YP = N1 + 32
ZZ = 4 * N2 * YP


def _yrow(src, n, part):
    return ((src * N2 + n) * 2 + part) * YP + 8 * ((n // 4 + 2 * part) % 4)


NF = (F + 127) // 128
KH = 512
LC = 64
KP = 24


MIDMEM, OMEM, FLAGS, FOLD, ORD = 0, 0, {}, 0, 0


def _words(m):
    u = np.ascontiguousarray(m).view(np.uint16).astype(np.uint32)
    return u[..., 0::2, :] | (u[..., 1::2, :] << 16)


def _perm_fwd():
    r = np.arange(N1)
    n1 = r // 2 + (N1 // 2) * (r % 2)
    return _words(_FWD[:, :, n1])


_FWD_P = _perm_fwd()
_INV_P = _words(_INV)


@jax.jit
def pallas_parallel_sum__ssm_conv_h3__dense_activation_gelu__prompt_kernel(
    A_q, A_k, A_v, A_shift_k, A_ssm_k, A_ssm_D, B_x, B_w1, B_b1, B_w2, B_b2,
):
    hbm = pl.BlockSpec(memory_space=pl.ANY)
    vmem = pl.BlockSpec(memory_space=pltpu.VMEM)
    return pl.pallas_call(
        _kernel,
        out_shape=jax.ShapeDtypeStruct((1, S, D), bf16),
        in_specs=[hbm, hbm, hbm, vmem, hbm, vmem, hbm, vmem, hbm, vmem, hbm, hbm,
                  pl.BlockSpec(memory_space=pltpu.SMEM)],
        out_specs=hbm,
        scratch_shapes=[
            pltpu.VMEM((S // 2, D), u32),
            pltpu.VMEM((G, S // 2 + 8, 128), u32),
            pltpu.VMEM((G, S // 2, 128), u32),
            pltpu.VMEM((D // 2, S), u32),
            pltpu.VMEM((F // 2, D), u32),
            pltpu.VMEM((F // 2, D), u32),
            pltpu.VMEM((N2, N1, N1), u32),
            pltpu.VMEM((N2, N1 // 2, 2 * N1), u32),
            pltpu.VMEM((G, KP * N1 // 2, 128), u32),
            pltpu.VMEM((G, N2, N1 // 2, 128), u32),
            pltpu.VMEM((G, S // 2, 128), u32),
            pltpu.VMEM((S // 2, D), u32),
            pltpu.VMEM((S // 2, F), u32),
            pltpu.VMEM((G, S, 128), f32),
            pltpu.VMEM((G, ZZ + S, 128), f32),
            pltpu.VMEM((1, F), f32),
            pltpu.VMEM((1, D), f32),
            pltpu.SemaphoreType.DMA((len(COPIES),)),
            pltpu.SemaphoreType.DMA((2,)),
        ],
        compiler_params=pltpu.CompilerParams(vmem_limit_bytes=100 * 2**20, flags=FLAGS),
    )(A_q, A_k, A_v, A_shift_k.T, A_ssm_k,
      A_ssm_D, B_w1.T, B_b1, B_w2, B_b2, _FWD_P, _INV_P, np.zeros((1,), np.int32))
```

```python
import contextlib

import jax
import jax.numpy as jnp
import numpy as np
import jax.experimental.pallas as pl
import jax.experimental.pallas.tpu as pltpu

S, D, F, KS = 2048, 640, 1728, 4
N1, N2 = 128, 16
G = D // 128
BM = 256
NB = S // BM
bf16, f32, u32 = jnp.bfloat16, jnp.float32, jnp.uint32


def _dft_mats():
    k1 = np.arange(N1)[None, :, None]
    n1 = np.arange(N1)[None, None, :]
    n2 = np.arange(N2)[:, None, None]
    ang = -2.0 * np.pi * (k1 + 0.25) * (N2 * n1 + n2) / S
    fr, fi = np.cos(ang), np.sin(ang)
    fwd = np.concatenate([fr, fi], axis=1)
    inv = np.stack([fr, fi], axis=2).reshape(N2, 2 * N1, N1)
    inv = np.transpose(inv, (0, 2, 1)) / S
    return fwd.astype(jnp.bfloat16), inv.astype(jnp.bfloat16)


_FWD, _INV = _dft_mats()

_C1, _S1, _R2 = float(np.cos(np.pi / 8)), float(np.sin(np.pi / 8)), float(np.sqrt(0.5))


def _bf4(a, b, c, d, sgn):
    t0 = (a[0] + c[0], a[1] + c[1])
    t1 = (a[0] - c[0], a[1] - c[1])
    t2 = (b[0] + d[0], b[1] + d[1])
    t3 = (b[0] - d[0], b[1] - d[1])
    o0 = (t0[0] + t2[0], t0[1] + t2[1])
    o2 = (t0[0] - t2[0], t0[1] - t2[1])
    p = (t1[0] + t3[1], t1[1] - t3[0])
    q = (t1[0] - t3[1], t1[1] + t3[0])
    return (o0, p, o2, q) if sgn < 0 else (o0, q, o2, p)


def _tw(x, e, sgn):
    r, i = x
    if e == 0:
        return x
    if e == 4:
        return (i, -r) if sgn < 0 else (-i, r)
    if e == 2:
        return ((r + i) * _R2, (i - r) * _R2) if sgn < 0 else ((r - i) * _R2, (r + i) * _R2)
    if e == 6:
        return ((i - r) * _R2, (r + i) * -_R2) if sgn < 0 else ((r + i) * -_R2, (r - i) * _R2)
    c = float(np.cos(2 * np.pi * e / 16))
    s = sgn * float(np.sin(2 * np.pi * e / 16))
    return (r * c - i * s, r * s + i * c)


_TWC = (16, 32, 24, 32)


def _lo(w):
    return pltpu.bitcast(w << 16, f32)


def _hi(w):
    return pltpu.bitcast(w & u32(0xFFFF0000), f32)


def _pack(a, b):
    return pltpu.pack_elementwise([a, b], packed_dtype=bf16).astype(u32)


def _gelu(h):
    c1 = 0.7978845608028654
    u = h * (c1 + (c1 * 0.044715) * (h * h))
    hh = 0.5 * h
    return hh + hh * jnp.tanh(u)


def _scope(name):
    return contextlib.nullcontext()


class _Fill:
    def __init__(self, steps):
        self.it = iter(steps)
        self.debt = 0

    def __call__(self, budget):
        self.debt += budget
        while self.debt > 0:
            c = next(self.it, None)
            if c is None:
                return
            self.debt -= c


def _kernel(q_hbm, k_hbm, v_hbm, sk_ref, ssm_hbm, d_ref, w1_hbm, b1_ref, w2_hbm, b2_ref,
            fwd_hbm, inv_hbm, zero_ref, o_hbm,
            q_buf, k_buf, v_buf, ssm_buf, w1_buf, w2_buf, fwd_buf, inv_buf,
            kt_buf, rhs_buf, y_buf, xn_buf, h_buf, acc, fb, b1_buf, b2_buf, sems, osems):
    qw, kw, vw, sw, w1w, w2w = (r.bitcast(u32) for r in (q_hbm, k_hbm, v_hbm, ssm_hbm, w1_hbm, w2_hbm))
    HB = BM // 2
    z0 = zero_ref[0]

    def copy(name):
        kind, i = name
        if kind == "q":
            rs = pl.ds(QCH[i] * HB, (QCH[i + 1] - QCH[i]) * HB)
            src, dst = qw.at[0, rs], q_buf.at[rs]
        elif kind == "w1":
            rs = pl.ds(WCH[i] // 2, (WCH[i + 1] - WCH[i]) // 2)
            src, dst = w1w.at[rs], w1_buf.at[rs]
        elif kind == "ssm":
            src, dst = sw.at[rows(i, 64)], ssm_buf.at[rows(i, 64)]
        elif kind == "k":
            src, dst = kw.at[0, :, rows(i, 128)], k_buf.at[i, pl.ds(8, S // 2)]
        elif kind == "v":
            src, dst = vw.at[0, :, rows(i, 128)], v_buf.at[i, pl.ds(0, S // 2)]
        else:
            src, dst = ((w2w, w2_buf), (fwd_hbm, fwd_buf), (inv_hbm, inv_buf))[i]
        return pltpu.make_async_copy(src, dst, sems.at[COPIES.index(name)])

    def start(*names):
        for name in names:
            copy(name).start()

    def wait(*names):
        for name in names:
            copy(name).wait()

    def conv_in(*groups):
        return [(kind, g) for g in groups for kind in ("ssm", "k", "v")]

    def rows(i, n):
        return pl.ds(i * n if isinstance(i, int) else pl.multiple_of(i * n, n), n)

    def norm(*blocks, cost=LC * 6):
        for i in blocks:
            for c in range(BM // LC):
                x = pltpu.bitcast(q_buf[rows(i * (BM // LC) + c, LC // 2), :], bf16).astype(f32)
                m = jnp.mean(x, axis=-1, keepdims=True)
                xc = x - m
                var = jnp.mean(xc * xc, axis=-1, keepdims=True)
                xn = (xc * jax.lax.rsqrt(var + 1e-5)).astype(bf16)
                xn_buf[rows(i * (BM // LC) + c, LC // 2), :] = pltpu.bitcast(xn, u32)
                yield cost

    def mm1(i, fill, cost, lo=0, hi=F):
        for f0 in range(lo, hi, 128):
            f1 = min(F, f0 + 128)
            xn = pltpu.bitcast(xn_buf[rows(i, HB), :], bf16)
            h = jax.lax.dot_general(xn, pltpu.bitcast(w1_buf[f0 // 2:f1 // 2, :], bf16),
                                    (((1,), (1,)), ((), ())), preferred_element_type=f32)
            h_buf[rows(i, HB), f0:f1] = pltpu.bitcast(_gelu(h + b1_buf[:, f0:f1]).astype(bf16), u32)
            fill(cost)

    def mm2(i, fill, cost, last=False):
        for g in range(G):
            ls = slice(g * 128, (g + 1) * 128)
            for f0 in range(0, F, KH):
                f1 = min(F, f0 + KH)
                h = pltpu.bitcast(h_buf[rows(i, HB), f0:f1], bf16)
                p = jnp.dot(h, pltpu.bitcast(w2_buf[f0 // 2:f1 // 2, ls], bf16),
                            preferred_element_type=f32)
                if last:
                    c = f0 // KH
                    if c:
                        p = acc[g, rows(i + z0, BM), :] + p
                    x = pltpu.bitcast(q_buf[rows(4 * (i + z0) + c, HB // 4), ls], bf16).astype(f32)
                    o = [p[r:r + BM // 4] for r in range(0, BM, BM // 4)]
                    o[c] = o[c] + (x + b2_buf[:, ls])
                    o = jnp.concatenate(o, axis=0)
                elif f0 == 0:
                    x = pltpu.bitcast(q_buf[rows(i, HB), ls], bf16).astype(f32)
                    o = p + (x + b2_buf[:, ls])
                else:
                    o = o + p
                if last and f1 == F:
                    gate(i, g, o)
                elif last or f1 == F:
                    acc[g, rows(i, BM), :] = o
                fill(cost * (f1 - f0) // 128)

    def prep(g):
        sk = sk_ref[:, g * 128:(g + 1) * 128].astype(f32)
        sk = [jnp.broadcast_to(sk[j:j + 1, :], (8, 128)) for j in range(KS)]
        rs = rows(g, 64)
        for a in range(8):
            lo, hi = (pltpu.bitcast(ssm_buf[rs, c:c + 128], bf16).astype(f32)
                      for c in (128 * a, 128 * a + S // 2))
            kt = _pack(lo, hi).T
            for j in range(8):
                kt_buf[g, pl.ds(KP * (8 * a + j), N2), :] = kt[N2 * j:N2 * (j + 1)]
            yield 96
            res = []
            for hf in range(2):
                base = a * 64 + hf * 512
                w = [kw_ld(g, base + 8 + m) for m in range(-2, 8)]
                ks = [f(x) for x in w for f in (_lo, _hi)]
                kv = []
                for m in range(8):
                    w = v_buf[g, pl.ds(base + m, 8, stride=8), :]
                    for p, vv in enumerate((_lo(w), _hi(w))):
                        n = 4 + 2 * m + p
                        s = (ks[n] * sk[0] + ks[n - 1] * sk[1]) + (ks[n - 2] * sk[2] + ks[n - 3] * sk[3])
                        kv.append(s * vv)
                res.append(kv)
                yield 172
            for n in range(N2):
                rhs_buf[g, n, pl.ds(a * 8, 8), :] = _pack(res[0][n], res[1][n])

    def kw_ld(g, r):
        return k_buf[g, pl.ds(r, 8, stride=8), :]

    def stage1(g, side=()):
        fill = _Fill(side)
        dd = d_ref[...].astype(f32).reshape(1, D)[:, g * 128:(g + 1) * 128]
        row = jax.lax.broadcasted_iota(jnp.int32, (8, 128), 0)
        dd = jnp.where(row == 0, jnp.broadcast_to(dd, (8, 128)), 0.0)
        for n in range(N2):
            kk = kt_buf[g, pl.ds(n, N1 // 2, stride=KP), :]
            if n == 0:
                top = _pack(_lo(kk[:8]) + dd, _hi(kk[:8]))
                kk = jnp.concatenate([top, kk[8:]], axis=0)
            rhs = pltpu.bitcast(jnp.concatenate([rhs_buf[g, n], kk], axis=1), bf16)
            y = jnp.dot(pltpu.bitcast(fwd_buf[n], bf16), rhs, preferred_element_type=f32)
            for src in range(2):
                for part in range(2):
                    fb[g, pl.ds(_yrow(src, n, part), N1), :] = (
                        y[part * N1:(part + 1) * N1, src * 128:(src + 1) * 128])
            fill(FILLB)
        fill(ALL)

    def middle(u0, nu):
        for u in range(nu):
            g = (u0 + u) // (N1 // 8)
            a = pl.multiple_of((u0 + u) % (N1 // 8) * 8, 8)

            ys = []
            for src in (1, 0):
                y = [[None] * 4 for _ in range(4)]
                for b in range(4):
                    x = [tuple(fb[g, pl.ds(a + _yrow(src, n, part), 8), :] for part in range(2))
                         for n in range(b, N2, 4)]
                    o = _bf4(*x, -1)
                    for c in range(4):
                        y[c][b] = _tw(o[c], b * c, -1)
                    yield _TWC[b]
                ys.append(y)
            w = [[None] * 4 for _ in range(4)]
            for c in range(4):
                sb = _bf4(*ys[0][c], -1)
                sa = _bf4(*ys[1][c], -1)
                pr = [(p[0] * q[0] - p[1] * q[1], p[0] * q[1] + p[1] * q[0]) for p, q in zip(sa, sb)]
                o = _bf4(*pr, 1)
                for e in range(4):
                    w[e][c] = _tw(o[e], c * e, 1)
                yield 56 + _TWC[c]
            for e in range(4):
                o = _bf4(*w[e], 1)
                for d in range(4):
                    fb[g, pl.ds(a + (ZZ + (e + 4 * d) * N1), 8), :] = pltpu.bitcast(_pack(*o[d]), f32)
                yield 20

    def inverse(g):
        for m in range(N2 // 2):
            y0, y1 = (jnp.dot(pltpu.bitcast(inv_buf[n], bf16), pltpu.bitcast(fb[g, pl.ds(ZZ + n * N1, N1), :], bf16),
                              preferred_element_type=f32) for n in (2 * m, 2 * m + 1))
            y_buf[g, pl.ds(m * YY, N1), :] = _pack(y0, y1)

    def out_copy(j):
        rs = pl.ds(OCH[j] * HB, (OCH[j + 1] - OCH[j]) * HB)
        return pltpu.make_async_copy(q_buf.at[rs], o_hbm.bitcast(u32).at[0, rs], osems.at[j])

    def gate(i, g, o):
        y = jnp.concatenate([y_buf[g, pl.ds(i * (HB // 8) + n, 8, stride=YY), :]
                             for n in range(HB // 8)], axis=0)
        y = pltpu.bitcast(y, bf16).astype(f32)
        xn = pltpu.bitcast(xn_buf[rows(i, HB), rows(g, 128)], bf16).astype(f32)
        q_buf[rows(i, HB), rows(g, 128)] = pltpu.bitcast((o + xn * y).astype(bf16), u32)

    def final(blocks):
        for i in blocks:
            for g in range(G):
                gate(i, g, acc[g, rows(i, BM), :])
                yield 150

    start(("q", 0))
    start(("w1", 0))
    for g in range(G):
        k_buf[g, pl.ds(0, 8), :] = jnp.zeros((8, 128), u32)
    b1_buf[...] = b1_ref[...].astype(f32).reshape(1, F)
    b2_buf[...] = b2_ref[...].astype(f32).reshape(1, D)
    with _scope("M0"):
        wait(("q", 0))
        start(("q", 1))
        start(("w1", 1))
        _Fill(norm(0))(ALL)
        wait(("w1", 0))
        mm1(0, _Fill(()), 0, WCH[0], WCH[1])
        wait(("q", 1))
        start(("w1", 2))
        _Fill(norm(1))(ALL)
        mm1(1, _Fill(()), 0, WCH[0], WCH[1])
        wait(("w1", 1))
        start(("q", 2))
        start(W2)
        for i in range(2):
            mm1(i, _Fill(()), 0, WCH[1], WCH[2])
        wait(("w1", 2))
        wait(("q", 2))
        start(("q", 3))
        fill = _Fill(norm(2, 3))
        for i in range(2):
            mm1(i, fill, FILLM, WCH[2], WCH[3])
        fill(ALL)
        wait(W2)
        wait(("q", 3))
        start(FWD, *conv_in(0, 1, 2))

    with _scope("A"):
        @pl.loop(0, 2)
        def _(i):
            @pl.when(i == 1)
            def _():
                start(("q", 4), *conv_in(3, 4))

            fill = _Fill(norm(4 + i))
            mm2(i, fill, 40)
            fill(ALL)
            mm1(i + 2, fill, 0)

    wait(FWD, *conv_in(0, 1, 2))
    start(INV)
    with _scope("prep0"):
        _Fill(prep(0))(ALL)
    with _scope("B"):
        for g in range(G - 1):
            if g == 2:
                wait(("q", 4), *conv_in(3, 4))
            stage1(g, prep(g + 1))

    with _scope("S4"):
        stage1(G - 1, norm(6, 7, cost=450))

    with _scope("C"):
        @pl.loop(0, G - 1)
        def _(g):
            fill = _Fill(middle(g * NU, NU))
            mm2(g + 2, fill, FILL2)
            mm1(g + 4, fill, FILL1)
            fill(ALL)

    wait(INV)
    with _scope("I"):
        pl.loop(0, G)(inverse)

    with _scope("E"):
        fill = _Fill(final([i for i in range(NB - 2)]))
        mm2(NB - 2, fill, FILLE, last=True)
        fill(ALL)

        out_copy(0).start()
        mm2(NB - 1, _Fill(()), 0, last=True)
        out_copy(1).start()
    out_copy(0).wait()
    out_copy(1).wait()


OCH = (0, NB - 1, NB)
FILL1, FILL2 = 335, 115
ALL = 10**9
WCH = (0, 256, 768, F)
QCH = (0, 1, 2, 4, 6, NB)
W2, FWD, INV = ("mat", 0), ("mat", 1), ("mat", 2)
COPIES = ([("q", i) for i in range(5)] + [("w1", i) for i in range(3)] + [W2, FWD, INV]
          + [(kind, g) for g in range(G) for kind in ("ssm", "k", "v")])
NU = G * (N1 // 8) // 4
YY = N1 + 1
YP = N1 + 32
ZZ = 4 * N2 * YP


def _yrow(src, n, part):
    return ((src * N2 + n) * 2 + part) * YP + 8 * ((n // 4 + 2 * part) % 4)


NF = (F + 127) // 128
KH = 512
LC = 32
KP = 17


FILLB, FILLE, FILLM = 225, 70, 250


def _words(m):
    u = np.ascontiguousarray(m).view(np.uint16).astype(np.uint32)
    return u[..., 0::2, :] | (u[..., 1::2, :] << 16)


def _perm_fwd():
    r = np.arange(N1)
    n1 = r // 2 + (N1 // 2) * (r % 2)
    return _words(_FWD[:, :, n1])


_FWD_P = _perm_fwd()
_INV_P = _words(_INV)


@jax.jit
def pallas_parallel_sum__ssm_conv_h3__dense_activation_gelu__prompt_kernel(
    A_q, A_k, A_v, A_shift_k, A_ssm_k, A_ssm_D, B_x, B_w1, B_b1, B_w2, B_b2,
):
    hbm = pl.BlockSpec(memory_space=pl.ANY)
    vmem = pl.BlockSpec(memory_space=pltpu.VMEM)
    return pl.pallas_call(
        _kernel,
        out_shape=jax.ShapeDtypeStruct((1, S, D), bf16),
        in_specs=[hbm, hbm, hbm, vmem, hbm, vmem, hbm, vmem, hbm, vmem, hbm, hbm,
                  pl.BlockSpec(memory_space=pltpu.SMEM)],
        out_specs=hbm,
        scratch_shapes=[
            pltpu.VMEM((S // 2, D), u32),
            pltpu.VMEM((G, S // 2 + 16, 128), u32),
            pltpu.VMEM((G, S // 2 + 8, 128), u32),
            pltpu.VMEM((D // 2, S), u32),
            pltpu.VMEM((F // 2, D), u32),
            pltpu.VMEM((F // 2, D), u32),
            pltpu.VMEM((N2, N1, N1), u32),
            pltpu.VMEM((N2, N1 // 2, 2 * N1), u32),
            pltpu.VMEM((G, KP * (N1 // 2 + 1), 128), u32),
            pltpu.VMEM((G, N2, N1 // 2, 128), u32),
            pltpu.VMEM((G, 9 * YY, 128), u32),
            pltpu.VMEM((S // 2, D), u32),
            pltpu.VMEM((S // 2, F), u32),
            pltpu.VMEM((G, S, 128), f32),
            pltpu.VMEM((G, ZZ + S, 128), f32),
            pltpu.VMEM((1, F), f32),
            pltpu.VMEM((1, D), f32),
            pltpu.SemaphoreType.DMA((len(COPIES),)),
            pltpu.SemaphoreType.DMA((2,)),
        ],
        compiler_params=pltpu.CompilerParams(vmem_limit_bytes=100 * 2**20),
    )(A_q, A_k, A_v, A_shift_k.T, A_ssm_k,
      A_ssm_D, B_w1.T, B_b1, B_w2, B_b2, _FWD_P, _INV_P, np.zeros((1,), np.int32))
```

```python
import contextlib

import jax
import jax.numpy as jnp
import numpy as np
import jax.experimental.pallas as pl
import jax.experimental.pallas.tpu as pltpu

S, D, F, KS = 2048, 640, 1728, 4
N1, N2 = 128, 16
G = D // 128
BM = 256
NB = S // BM
bf16, f32, u32 = jnp.bfloat16, jnp.float32, jnp.uint32


def _dft_mats():
    k1 = np.arange(N1)[None, :, None]
    n1 = np.arange(N1)[None, None, :]
    n2 = np.arange(N2)[:, None, None]
    ang = -2.0 * np.pi * (k1 + 0.25) * (N2 * n1 + n2) / S
    fr, fi = np.cos(ang), np.sin(ang)
    fwd = np.concatenate([fr, fi], axis=1)
    inv = np.stack([fr, fi], axis=2)[:, :N1 // 2].reshape(N2, N1, N1)
    inv = np.transpose(inv, (0, 2, 1)) / S
    inv = np.concatenate([inv[:, 0::2], inv[:, 1::2]], axis=1)
    return fwd.astype(jnp.bfloat16), inv.astype(jnp.bfloat16)


_FWD, _INV = _dft_mats()

_C1, _S1, _R2 = float(np.cos(np.pi / 8)), float(np.sin(np.pi / 8)), float(np.sqrt(0.5))


def _bf4(a, b, c, d, sgn):
    t0 = (a[0] + c[0], a[1] + c[1])
    t1 = (a[0] - c[0], a[1] - c[1])
    t2 = (b[0] + d[0], b[1] + d[1])
    t3 = (b[0] - d[0], b[1] - d[1])
    o0 = (t0[0] + t2[0], t0[1] + t2[1])
    o2 = (t0[0] - t2[0], t0[1] - t2[1])
    p = (t1[0] + t3[1], t1[1] - t3[0])
    q = (t1[0] - t3[1], t1[1] + t3[0])
    return (o0, p, o2, q) if sgn < 0 else (o0, q, o2, p)


def _tw(x, e, sgn):
    r, i = x
    if e == 0:
        return x
    if e == 4:
        return (i, -r) if sgn < 0 else (-i, r)
    if e == 2:
        return ((r + i) * _R2, (i - r) * _R2) if sgn < 0 else ((r - i) * _R2, (r + i) * _R2)
    if e == 6:
        return ((i - r) * _R2, (r + i) * -_R2) if sgn < 0 else ((r + i) * -_R2, (r - i) * _R2)
    c = float(np.cos(2 * np.pi * e / 16))
    s = sgn * float(np.sin(2 * np.pi * e / 16))
    return (r * c - i * s, r * s + i * c)


_TWC = (16, 32, 24, 32)


def _lo(w):
    return pltpu.bitcast(w << 16, f32)


def _hi(w):
    return pltpu.bitcast(w & u32(0xFFFF0000), f32)


def _pack(a, b):
    return pltpu.pack_elementwise([a, b], packed_dtype=bf16).astype(u32)


def _gelu(h):
    c1 = 0.7978845608028654
    u = h * (c1 + (c1 * 0.044715) * (h * h))
    hh = 0.5 * h
    return hh + hh * jnp.tanh(u)


def _scope(name):
    return contextlib.nullcontext()


class _Fill:
    def __init__(self, steps):
        self.it = iter(steps)
        self.debt = 0

    def __call__(self, budget):
        self.debt += budget
        while self.debt > 0:
            c = next(self.it, None)
            if c is None:
                return
            self.debt -= c


def _kernel(q_hbm, k_hbm, v_hbm, sk_ref, ssm_hbm, d_ref, w1_hbm, b1_ref, w2_hbm, b2_ref,
            fwd_hbm, inv_hbm, zero_ref, o_hbm,
            q_buf, k_buf, v_buf, ssm_buf, w1_buf, w2_buf, fwd_buf, inv_buf,
            kt_buf, rhs_buf, y_buf, xn_buf, h_buf, acc, fb, b1_buf, b2_buf, sems, osems):
    qw, kw, vw, sw, w1w, w2w = (r.bitcast(u32) for r in (q_hbm, k_hbm, v_hbm, ssm_hbm, w1_hbm, w2_hbm))
    HB = BM // 2
    z0 = zero_ref[0]

    def copy(name):
        kind, i = name
        if kind == "q":
            rs = pl.ds(QCH[i] * HB, (QCH[i + 1] - QCH[i]) * HB)
            src, dst = qw.at[0, rs], q_buf.at[rs]
        elif kind == "w1":
            rs = pl.ds(WCH[i] // 2, (WCH[i + 1] - WCH[i]) // 2)
            src, dst = w1w.at[rs], w1_buf.at[rs]
        elif kind == "ssm":
            src, dst = sw.at[rows(i, 64)], ssm_buf.at[rows(i, 64)]
        elif kind == "k":
            src, dst = kw.at[0, :, rows(i, 128)], k_buf.at[i, pl.ds(8, S // 2)]
        elif kind == "v":
            src, dst = vw.at[0, :, rows(i, 128)], v_buf.at[i, pl.ds(0, S // 2)]
        else:
            src, dst = ((w2w, w2_buf), (fwd_hbm, fwd_buf), (inv_hbm, inv_buf))[i]
        return pltpu.make_async_copy(src, dst, sems.at[COPIES.index(name)])

    def start(*names):
        for name in names:
            copy(name).start()

    def wait(*names):
        for name in names:
            copy(name).wait()

    def conv_in(*groups):
        return [(kind, g) for g in groups for kind in ("ssm", "k", "v")]

    def rows(i, n):
        return pl.ds(i * n if isinstance(i, int) else pl.multiple_of(i * n, n), n)

    def norm(*blocks, cost=LC * 6):
        for i in blocks:
            for c in range(BM // LC):
                x = pltpu.bitcast(q_buf[rows(i * (BM // LC) + c, LC // 2), :], bf16).astype(f32)
                m = jnp.mean(x, axis=-1, keepdims=True)
                xc = x - m
                var = jnp.mean(xc * xc, axis=-1, keepdims=True)
                xn = (xc * jax.lax.rsqrt(var + 1e-5)).astype(bf16)
                xn_buf[rows(i * (BM // LC) + c, LC // 2), :] = pltpu.bitcast(xn, u32)
                yield cost

    def mm1(i, fill, cost, lo=0, hi=F):
        for f0 in range(lo, hi, 128):
            f1 = min(F, f0 + 128)
            xn = pltpu.bitcast(xn_buf[rows(i, HB), :], bf16)
            h = jax.lax.dot_general(xn, pltpu.bitcast(w1_buf[f0 // 2:f1 // 2, :], bf16),
                                    (((1,), (1,)), ((), ())), preferred_element_type=f32)
            h_buf[rows(i, HB), f0:f1] = pltpu.bitcast(_gelu(h + b1_buf[:, f0:f1]).astype(bf16), u32)
            fill(cost)

    def mm2(i, fill, cost, last=False):
        for g in range(G):
            ls = slice(g * 128, (g + 1) * 128)
            for f0 in range(0, F, KH):
                f1 = min(F, f0 + KH)
                h = pltpu.bitcast(h_buf[rows(i, HB), f0:f1], bf16)
                p = jnp.dot(h, pltpu.bitcast(w2_buf[f0 // 2:f1 // 2, ls], bf16),
                            preferred_element_type=f32)
                if last:
                    c = f0 // KH
                    if c:
                        p = acc[g, rows(i + z0, BM), :] + p
                    x = pltpu.bitcast(q_buf[rows(4 * (i + z0) + c, HB // 4), ls], bf16).astype(f32)
                    o = [p[r:r + BM // 4] for r in range(0, BM, BM // 4)]
                    o[c] = o[c] + (x + b2_buf[:, ls])
                    o = jnp.concatenate(o, axis=0)
                elif f0 == 0:
                    x = pltpu.bitcast(q_buf[rows(i, HB), ls], bf16).astype(f32)
                    o = p + (x + b2_buf[:, ls])
                else:
                    o = o + p
                if last and f1 == F:
                    gate(i, g, o)
                elif last or f1 == F:
                    acc[g, rows(i, BM), :] = o
                fill(cost * (f1 - f0) // 128)

    def prep(g):
        sk = sk_ref[:, g * 128:(g + 1) * 128].astype(f32)
        sk = [jnp.broadcast_to(sk[j:j + 1, :], (8, 128)) for j in range(KS)]
        rs = rows(g, 64)
        for a in range(8):
            lo, hi = (pltpu.bitcast(ssm_buf[rs, c:c + 128], bf16).astype(f32)
                      for c in (128 * a, 128 * a + S // 2))
            kt = _pack(lo, hi).T
            for j in range(8):
                kt_buf[g, pl.ds(KP * (8 * a + j), N2), :] = kt[N2 * j:N2 * (j + 1)]
            yield 96
            res = []
            for hf in range(2):
                base = a * 64 + hf * 512
                w = [kw_ld(g, base + 8 + m) for m in range(-2, 8)]
                ks = [f(x) for x in w for f in (_lo, _hi)]
                kv = []
                for m in range(8):
                    w = v_buf[g, pl.ds(base + m, 8, stride=8), :]
                    for p, vv in enumerate((_lo(w), _hi(w))):
                        n = 4 + 2 * m + p
                        s = (ks[n] * sk[0] + ks[n - 1] * sk[1]) + (ks[n - 2] * sk[2] + ks[n - 3] * sk[3])
                        kv.append(s * vv)
                res.append(kv)
                yield 172
            for n in range(N2):
                rhs_buf[g, n, pl.ds(a * 8, 8), :] = _pack(res[0][n], res[1][n])

    def kw_ld(g, r):
        return k_buf[g, pl.ds(r, 8, stride=8), :]

    def stage1(g, side=()):
        fill = _Fill(side)
        dd = d_ref[...].astype(f32).reshape(1, D)[:, g * 128:(g + 1) * 128]
        row = jax.lax.broadcasted_iota(jnp.int32, (8, 128), 0)
        dd = jnp.where(row == 0, jnp.broadcast_to(dd, (8, 128)), 0.0)
        for n in range(N2):
            kk = kt_buf[g, pl.ds(n, N1 // 2, stride=KP), :]
            if n == 0:
                top = _pack(_lo(kk[:8]) + dd, _hi(kk[:8]))
                kk = jnp.concatenate([top, kk[8:]], axis=0)
            rhs = pltpu.bitcast(jnp.concatenate([rhs_buf[g, n], kk], axis=1), bf16)
            y = jnp.dot(pltpu.bitcast(fwd_buf[n], bf16), rhs, preferred_element_type=f32)
            for src in range(2):
                for part in range(2):
                    fb[g, pl.ds(_yrow(src, n, part), N1), :] = (
                        y[part * N1:(part + 1) * N1, src * 128:(src + 1) * 128])
            fill(FILLB)
        fill(ALL)

    def spectrum_product(g, a):
        ys = []
        for src in (1, 0):
            y = [[None] * 4 for _ in range(4)]
            for b in range(4):
                x = [tuple(fb[g, pl.ds(a + _yrow(src, n, part), 8), :] for part in range(2))
                     for n in range(b, N2, 4)]
                o = _bf4(*x, -1)
                for c in range(4):
                    y[c][b] = _tw(o[c], b * c, -1)
                yield _TWC[b]
            ys.append(y)
        w = [[None] * 4 for _ in range(4)]
        for c in range(4):
            sb = _bf4(*ys[0][c], -1)
            sa = _bf4(*ys[1][c], -1)
            pr = [(p[0] * q[0] - p[1] * q[1], p[0] * q[1] + p[1] * q[0]) for p, q in zip(sa, sb)]
            o = _bf4(*pr, 1)
            for e in range(4):
                w[e][c] = _tw(o[e], c * e, 1)
            yield 56 + _TWC[c]
        return w

    def middle(u0, nu):
        for u in range(nu):
            g = (u0 + u) // (N1 // 8)
            a = pl.multiple_of((u0 + u) % (N1 // 8) * 8, 8)
            w = yield from spectrum_product(g, a)
            for e in range(4):
                o = _bf4(*w[e], 1)
                for d in range(4):
                    for part in range(2):
                        fb[g, pl.ds(a + _yrow(2, e + 4 * d, part), 8), :] = o[d][part]
                yield 20

    def inverse(g):
        H = N1 // 2
        for m in range(N2 // 2):
            zs = []
            for n in (2 * m, 2 * m + 1):
                lo, hi = (tuple(fb[g, pl.ds(_yrow(2, n, part) + r, H), :] for part in range(2))
                          for r in (0, H))
                t = _tw(hi, n / 2, 1)
                zs.append((_pack(lo[0] + t[0], lo[1] + t[1]), _pack(lo[0] - t[0], lo[1] - t[1])))
            for par in range(2):
                y0, y1 = (jnp.dot(pltpu.bitcast(inv_buf[2 * m + j, rows(par, H // 2), :], bf16),
                                  pltpu.bitcast(zs[j][par], bf16), preferred_element_type=f32)
                          for j in range(2))
                y_buf[g, pl.ds(m * YY + par * H, H), :] = _pack(y0, y1)

    def out_copy(j):
        rs = pl.ds(OCH[j] * HB, (OCH[j + 1] - OCH[j]) * HB)
        return pltpu.make_async_copy(q_buf.at[rs], o_hbm.bitcast(u32).at[0, rs], osems.at[j])

    def gate(i, g, o):
        y = jnp.concatenate([y_buf[g, pl.ds(i * (HB // 16) + (n // 2 + n % 2 * (N1 // 2)), 8, stride=YY), :]
                             for n in range(HB // 8)], axis=0)
        y = pltpu.bitcast(y, bf16).astype(f32)
        xn = pltpu.bitcast(xn_buf[rows(i, HB), rows(g, 128)], bf16).astype(f32)
        q_buf[rows(i, HB), rows(g, 128)] = pltpu.bitcast((o + xn * y).astype(bf16), u32)

    def final(blocks):
        for i in blocks:
            for g in range(G):
                gate(i, g, acc[g, rows(i, BM), :])
                yield 150

    start(("q", 0))
    start(("w1", 0))
    for g in range(G):
        k_buf[g, pl.ds(0, 8), :] = jnp.zeros((8, 128), u32)
    b1_buf[...] = b1_ref[...].astype(f32).reshape(1, F)
    b2_buf[...] = b2_ref[...].astype(f32).reshape(1, D)
    with _scope("M0"):
        wait(("q", 0))
        start(("q", 1))
        start(("w1", 1))
        _Fill(norm(0))(ALL)
        wait(("w1", 0))
        mm1(0, _Fill(()), 0, WCH[0], WCH[1])
        wait(("q", 1))
        start(("w1", 2))
        _Fill(norm(1))(ALL)
        mm1(1, _Fill(()), 0, WCH[0], WCH[1])
        wait(("w1", 1))
        start(("q", 2))
        start(W2)
        for i in range(2):
            mm1(i, _Fill(()), 0, WCH[1], WCH[2])
        wait(("w1", 2))
        wait(("q", 2))
        start(("q", 3))
        fill = _Fill(norm(2, 3))
        for i in range(2):
            mm1(i, fill, FILLM, WCH[2], WCH[3])
        fill(ALL)
        wait(W2)
        wait(("q", 3))
        start(FWD, *conv_in(0, 1, 2))

    with _scope("A"):
        @pl.loop(0, 2)
        def _(i):
            @pl.when(i == 1)
            def _():
                start(("q", 4), *conv_in(3, 4))

            fill = _Fill(norm(4 + i))
            mm2(i, fill, 40)
            fill(ALL)
            mm1(i + 2, fill, 0)

    wait(FWD, *conv_in(0, 1, 2))
    start(INV)
    with _scope("prep0"):
        _Fill(prep(0))(ALL)
    with _scope("B"):
        for g in range(G - 1):
            if g == 2:
                wait(("q", 4), *conv_in(3, 4))
            stage1(g, prep(g + 1))

    with _scope("S4"):
        stage1(G - 1, norm(6, 7, cost=450))

    with _scope("C"):
        @pl.loop(0, G - 1)
        def _(g):
            fill = _Fill(middle(g * NU, NU))
            mm2(g + 2, fill, FILL2)
            mm1(g + 4, fill, FILL1)
            fill(ALL)

    wait(INV)
    with _scope("I"):
        if UNI:
            for g in range(G):
                inverse(g)
        else:
            pl.loop(0, G)(inverse)

    with _scope("E"):
        fill = _Fill(final([i for i in range(NB - 2)]))
        mm2(NB - 2, fill, FILLE, last=True)
        fill(ALL)

        out_copy(0).start()
        mm2(NB - 1, _Fill(()), 0, last=True)
        out_copy(1).start()
    out_copy(0).wait()
    out_copy(1).wait()


OCH = (0, NB - 1, NB)
FILL1, FILL2 = 335, 115
ALL = 10**9
WCH = (0, 256, 768, F)
QCH = (0, 1, 2, 4, 6, NB)
W2, FWD, INV = ("mat", 0), ("mat", 1), ("mat", 2)
COPIES = ([("q", i) for i in range(5)] + [("w1", i) for i in range(3)] + [W2, FWD, INV]
          + [(kind, g) for g in range(G) for kind in ("ssm", "k", "v")])
NU = G * (N1 // 8) // 4
YY = N1 + 1
YP = N1 + 32


def _yrow(src, n, part):
    return ((src * N2 + n) * 2 + part) * YP + 8 * ((n // 4 + 2 * part) % 4)


NF = (F + 127) // 128
KH = 512
LC = 32
KP = 17


FILLB, FILLE, FILLM = 225, 70, 250
UNI = 0


def _words(m):
    u = np.ascontiguousarray(m).view(np.uint16).astype(np.uint32)
    return u[..., 0::2, :] | (u[..., 1::2, :] << 16)


def _perm_fwd():
    r = np.arange(N1)
    n1 = r // 2 + (N1 // 2) * (r % 2)
    return _words(_FWD[:, :, n1])


_FWD_P = _perm_fwd()
_INV_P = _words(_INV)


@jax.jit
def pallas_parallel_sum__ssm_conv_h3__dense_activation_gelu__prompt_kernel(
    A_q, A_k, A_v, A_shift_k, A_ssm_k, A_ssm_D, B_x, B_w1, B_b1, B_w2, B_b2,
):
    hbm = pl.BlockSpec(memory_space=pl.ANY)
    vmem = pl.BlockSpec(memory_space=pltpu.VMEM)
    return pl.pallas_call(
        _kernel,
        out_shape=jax.ShapeDtypeStruct((1, S, D), bf16),
        in_specs=[hbm, hbm, hbm, vmem, hbm, vmem, hbm, vmem, hbm, vmem, hbm, hbm,
                  pl.BlockSpec(memory_space=pltpu.SMEM)],
        out_specs=hbm,
        scratch_shapes=[
            pltpu.VMEM((S // 2, D), u32),
            pltpu.VMEM((G, S // 2 + 16, 128), u32),
            pltpu.VMEM((G, S // 2 + 8, 128), u32),
            pltpu.VMEM((D // 2, S), u32),
            pltpu.VMEM((F // 2, D), u32),
            pltpu.VMEM((F // 2, D), u32),
            pltpu.VMEM((N2, N1, N1), u32),
            pltpu.VMEM((N2, N1 // 2, N1), u32),
            pltpu.VMEM((G, KP * (N1 // 2 + 1), 128), u32),
            pltpu.VMEM((G, N2, N1 // 2, 128), u32),
            pltpu.VMEM((G, 9 * YY, 128), u32),
            pltpu.VMEM((S // 2, D), u32),
            pltpu.VMEM((S // 2, F), u32),
            pltpu.VMEM((G, S, 128), f32),
            pltpu.VMEM((G, 6 * N2 * YP, 128), f32),
            pltpu.VMEM((1, F), f32),
            pltpu.VMEM((1, D), f32),
            pltpu.SemaphoreType.DMA((len(COPIES),)),
            pltpu.SemaphoreType.DMA((2,)),
        ],
        compiler_params=pltpu.CompilerParams(vmem_limit_bytes=100 * 2**20),
    )(A_q, A_k, A_v, A_shift_k.T, A_ssm_k,
      A_ssm_D, B_w1.T, B_b1, B_w2, B_b2, _FWD_P, _INV_P, np.zeros((1,), np.int32))
```

```python
import contextlib

import jax
import jax.numpy as jnp
import numpy as np
import jax.experimental.pallas as pl
import jax.experimental.pallas.tpu as pltpu

S, D, F, KS = 2048, 640, 1728, 4
N1, N2 = 128, 16
G = D // 128
BM = 256
NB = S // BM
bf16, f32, u32 = jnp.bfloat16, jnp.float32, jnp.uint32


def _dft_mats():
    k1 = np.arange(N1)[None, :, None]
    n1 = np.arange(N1)[None, None, :]
    n2 = np.arange(N2)[:, None, None]
    ang = -2.0 * np.pi * (k1 + 0.25) * (N2 * n1 + n2) / S
    fr, fi = np.cos(ang), np.sin(ang)
    fwd = np.concatenate([fr, fi], axis=1)
    inv = np.stack([fr, fi], axis=2)[:, :N1 // 2].reshape(N2, N1, N1)
    inv = np.transpose(inv, (0, 2, 1)) / S
    inv = np.concatenate([inv[:, 0::2], inv[:, 1::2]], axis=1)
    return fwd.astype(jnp.bfloat16), inv.astype(jnp.bfloat16)


_FWD, _INV = _dft_mats()

_C1, _S1, _R2 = float(np.cos(np.pi / 8)), float(np.sin(np.pi / 8)), float(np.sqrt(0.5))


def _bf4(a, b, c, d, sgn):
    t0 = (a[0] + c[0], a[1] + c[1])
    t1 = (a[0] - c[0], a[1] - c[1])
    t2 = (b[0] + d[0], b[1] + d[1])
    t3 = (b[0] - d[0], b[1] - d[1])
    o0 = (t0[0] + t2[0], t0[1] + t2[1])
    o2 = (t0[0] - t2[0], t0[1] - t2[1])
    p = (t1[0] + t3[1], t1[1] - t3[0])
    q = (t1[0] - t3[1], t1[1] + t3[0])
    return (o0, p, o2, q) if sgn < 0 else (o0, q, o2, p)


def _tw(x, e, sgn):
    r, i = x
    if e == 0:
        return x
    if e == 4:
        return (i, -r) if sgn < 0 else (-i, r)
    if e == 2:
        return ((r + i) * _R2, (i - r) * _R2) if sgn < 0 else ((r - i) * _R2, (r + i) * _R2)
    if e == 6:
        return ((i - r) * _R2, (r + i) * -_R2) if sgn < 0 else ((r + i) * -_R2, (r - i) * _R2)
    c = float(np.cos(2 * np.pi * e / 16))
    s = sgn * float(np.sin(2 * np.pi * e / 16))
    return (r * c - i * s, r * s + i * c)


_TWC = (16, 32, 24, 32)


def _lo(w):
    return pltpu.bitcast(w << 16, f32)


def _hi(w):
    return pltpu.bitcast(w & u32(0xFFFF0000), f32)


def _pack(a, b):
    return pltpu.pack_elementwise([a, b], packed_dtype=bf16).astype(u32)


def _gelu(h):
    c1 = 0.7978845608028654
    u = h * (c1 + (c1 * 0.044715) * (h * h))
    hh = 0.5 * h
    return hh + hh * jnp.tanh(u)


def _scope(name):
    return contextlib.nullcontext()


class _Fill:
    def __init__(self, steps):
        self.it = iter(steps)
        self.debt = 0

    def __call__(self, budget):
        self.debt += budget
        while self.debt > 0:
            c = next(self.it, None)
            if c is None:
                return
            self.debt -= c


def _kernel(q_hbm, k_hbm, v_hbm, sk_ref, ssm_hbm, d_ref, w1_hbm, b1_ref, w2_hbm, b2_ref,
            fwd_hbm, inv_hbm, zero_ref, o_hbm,
            q_buf, k_buf, v_buf, ssm_buf, w1_buf, w2_buf, fwd_buf, inv_buf,
            kt_buf, rhs_buf, y_buf, xn_buf, h_buf, acc, fb, b1_buf, bt_buf, b2_buf, sems, osems):
    qw, kw, vw, sw, w1w, w2w = (r.bitcast(u32) for r in (q_hbm, k_hbm, v_hbm, ssm_hbm, w1_hbm, w2_hbm))
    HB = BM // 2
    z0 = zero_ref[0]

    def copy(name):
        kind, i = name
        if kind == "q":
            rs = pl.ds(QCH[i] * HB, (QCH[i + 1] - QCH[i]) * HB)
            src, dst = qw.at[0, rs], q_buf.at[rs]
        elif kind == "w1":
            rs = pl.ds(WCH[i] // 2, (WCH[i + 1] - WCH[i]) // 2)
            src, dst = w1w.at[rs], w1_buf.at[rs]
        elif kind == "ssm":
            src, dst = sw.at[rows(i, 64)], ssm_buf.at[rows(i, 64)]
        elif kind == "k":
            src, dst = kw.at[0, :, rows(i, 128)], k_buf.at[i, pl.ds(8, S // 2)]
        elif kind == "v":
            src, dst = vw.at[0, :, rows(i, 128)], v_buf.at[i, pl.ds(0, S // 2)]
        else:
            src, dst = ((w2w, w2_buf), (fwd_hbm, fwd_buf), (inv_hbm, inv_buf))[i]
        return pltpu.make_async_copy(src, dst, sems.at[COPIES.index(name)])

    def start(*names):
        for name in names:
            copy(name).start()

    def wait(*names):
        for name in names:
            copy(name).wait()

    def conv_in(*groups):
        return [(kind, g) for g in groups for kind in ("ssm", "k", "v")]

    def rows(i, n):
        return pl.ds(i * n if isinstance(i, int) else pl.multiple_of(i * n, n), n)

    def norm(*blocks, cost=LC * 6):
        for i in blocks:
            for c in range(BM // LC):
                x = pltpu.bitcast(q_buf[rows(i * (BM // LC) + c, LC // 2), :], bf16).astype(f32)
                m = jnp.mean(x, axis=-1, keepdims=True)
                xc = x - m
                var = jnp.mean(xc * xc, axis=-1, keepdims=True)
                xn = (xc * jax.lax.rsqrt(var + 1e-5)).astype(bf16)
                xn_buf[rows(i * (BM // LC) + c, LC // 2), :] = pltpu.bitcast(xn, u32)
                yield cost

    def mm1(i, fill, cost, lo=0, hi=F):
        for f0 in range(lo, hi, 128):
            f1 = min(F, f0 + 128)
            xn = pltpu.bitcast(xn_buf[rows(i, HB), :], bf16)
            w = pltpu.bitcast(w1_buf[f0 // 2:f1 // 2, :], bf16)
            nt = (((1,), (1,)), ((), ()))
            if f1 - f0 == 128:
                h = jax.lax.dot_general(xn, w, nt, preferred_element_type=f32)
                h = _gelu(h + b1_buf[:, f0:f1])
            else:
                h = jax.lax.dot_general(w, xn, nt, preferred_element_type=f32)
                h = _gelu(h + jnp.tile(bt_buf[...], (1, BM // 128))).T
            h_buf[rows(i, HB), f0:f1] = pltpu.bitcast(h.astype(bf16), u32)
            fill(cost)

    def mm2(i, fill, cost, last=False):
        for g in range(G):
            ls = slice(g * 128, (g + 1) * 128)
            for f0 in range(0, F, KH):
                f1 = min(F, f0 + KH)
                h = pltpu.bitcast(h_buf[rows(i, HB), f0:f1], bf16)
                p = jnp.dot(h, pltpu.bitcast(w2_buf[f0 // 2:f1 // 2, ls], bf16),
                            preferred_element_type=f32)
                if last:
                    c = f0 // KH
                    if c:
                        p = acc[g, rows(i + z0, BM), :] + p
                    x = pltpu.bitcast(q_buf[rows(4 * (i + z0) + c, HB // 4), ls], bf16).astype(f32)
                    o = [p[r:r + BM // 4] for r in range(0, BM, BM // 4)]
                    o[c] = o[c] + (x + b2_buf[:, ls])
                    o = jnp.concatenate(o, axis=0)
                elif f0 == 0:
                    x = pltpu.bitcast(q_buf[rows(i, HB), ls], bf16).astype(f32)
                    o = p + (x + b2_buf[:, ls])
                else:
                    o = o + p
                if last and f1 == F:
                    gate(i, g, o)
                elif last or f1 == F:
                    acc[g, rows(i, BM), :] = o
                fill(cost * (f1 - f0) // 128)

    def prep(g):
        sk = sk_ref[:, g * 128:(g + 1) * 128].astype(f32)
        sk = [jnp.broadcast_to(sk[j:j + 1, :], (8, 128)) for j in range(KS)]
        rs = rows(g, 64)
        for a in range(8):
            lo, hi = (pltpu.bitcast(ssm_buf[rs, c:c + 128], bf16).astype(f32)
                      for c in (128 * a, 128 * a + S // 2))
            kt = _pack(lo, hi).T
            for j in range(8):
                kt_buf[g, pl.ds(KP * (8 * a + j), N2), :] = kt[N2 * j:N2 * (j + 1)]
            yield 96
            res = []
            for hf in range(2):
                base = a * 64 + hf * 512
                w = [kw_ld(g, base + 8 + m) for m in range(-2, 8)]
                ks = [f(x) for x in w for f in (_lo, _hi)]
                kv = []
                for m in range(8):
                    w = v_buf[g, pl.ds(base + m, 8, stride=8), :]
                    for p, vv in enumerate((_lo(w), _hi(w))):
                        n = 4 + 2 * m + p
                        s = (ks[n] * sk[0] + ks[n - 1] * sk[1]) + (ks[n - 2] * sk[2] + ks[n - 3] * sk[3])
                        kv.append(s * vv)
                res.append(kv)
                yield 172
            for n in range(N2):
                rhs_buf[g, n, pl.ds(a * 8, 8), :] = _pack(res[0][n], res[1][n])

    def kw_ld(g, r):
        return k_buf[g, pl.ds(r, 8, stride=8), :]

    def stage1(g, side=()):
        fill = _Fill(side)
        dd = d_ref[...].astype(f32).reshape(1, D)[:, g * 128:(g + 1) * 128]
        row = jax.lax.broadcasted_iota(jnp.int32, (8, 128), 0)
        dd = jnp.where(row == 0, jnp.broadcast_to(dd, (8, 128)), 0.0)
        for n in range(N2):
            kk = kt_buf[g, pl.ds(n, N1 // 2, stride=KP), :]
            if n == 0:
                top = _pack(_lo(kk[:8]) + dd, _hi(kk[:8]))
                kk = jnp.concatenate([top, kk[8:]], axis=0)
            rhs = pltpu.bitcast(jnp.concatenate([rhs_buf[g, n], kk], axis=1), bf16)
            y = jnp.dot(pltpu.bitcast(fwd_buf[n], bf16), rhs, preferred_element_type=f32)
            for src in range(2):
                for part in range(2):
                    fb[g, pl.ds(_yrow(src, n, part), N1), :] = (
                        y[part * N1:(part + 1) * N1, src * 128:(src + 1) * 128])
            fill(FILLB)
        fill(ALL)

    def spectrum_product(g, a):
        ys = []
        for src in (1, 0):
            y = [[None] * 4 for _ in range(4)]
            for b in range(4):
                x = [tuple(fb[g, pl.ds(a + _yrow(src, n, part), 8), :] for part in range(2))
                     for n in range(b, N2, 4)]
                o = _bf4(*x, -1)
                for c in range(4):
                    y[c][b] = _tw(o[c], b * c, -1)
                yield _TWC[b]
            ys.append(y)
        w = [[None] * 4 for _ in range(4)]
        for c in range(4):
            sb = _bf4(*ys[0][c], -1)
            sa = _bf4(*ys[1][c], -1)
            pr = [(p[0] * q[0] - p[1] * q[1], p[0] * q[1] + p[1] * q[0]) for p, q in zip(sa, sb)]
            o = _bf4(*pr, 1)
            for e in range(4):
                w[e][c] = _tw(o[e], c * e, 1)
            yield 56 + _TWC[c]
        return w

    def middle(u0, nu):
        for u in range(nu):
            g = (u0 + u) // (N1 // 8)
            a = pl.multiple_of((u0 + u) % (N1 // 8) * 8, 8)
            w = yield from spectrum_product(g, a)
            for e in range(4):
                o = _bf4(*w[e], 1)
                for d in range(4):
                    for part in range(2):
                        fb[g, pl.ds(a + _yrow(2, e + 4 * d, part), 8), :] = o[d][part]
                yield 20

    def inverse(g):
        H = N1 // 2
        for m in range(N2 // 2):
            zs = []
            for n in (2 * m, 2 * m + 1):
                lo, hi = (tuple(fb[g, pl.ds(_yrow(2, n, part) + r, H), :] for part in range(2))
                          for r in (0, H))
                t = _tw(hi, n / 2, 1)
                zs.append((_pack(lo[0] + t[0], lo[1] + t[1]), _pack(lo[0] - t[0], lo[1] - t[1])))
            for par in range(2):
                y0, y1 = (jnp.dot(pltpu.bitcast(inv_buf[2 * m + j, rows(par, H // 2), :], bf16),
                                  pltpu.bitcast(zs[j][par], bf16), preferred_element_type=f32)
                          for j in range(2))
                y_buf[g, pl.ds(m * YY + par * H, H), :] = _pack(y0, y1)

    def out_copy(j):
        rs = pl.ds(OCH[j] * HB, (OCH[j + 1] - OCH[j]) * HB)
        return pltpu.make_async_copy(q_buf.at[rs], o_hbm.bitcast(u32).at[0, rs], osems.at[j])

    def gate(i, g, o):
        y = jnp.concatenate([y_buf[g, pl.ds(i * (HB // 16) + (n // 2 + n % 2 * (N1 // 2)), 8, stride=YY), :]
                             for n in range(HB // 8)], axis=0)
        y = pltpu.bitcast(y, bf16).astype(f32)
        xn = pltpu.bitcast(xn_buf[rows(i, HB), rows(g, 128)], bf16).astype(f32)
        q_buf[rows(i, HB), rows(g, 128)] = pltpu.bitcast((o + xn * y).astype(bf16), u32)

    def final(blocks):
        for i in blocks:
            for g in range(G):
                gate(i, g, acc[g, rows(i, BM), :])
                yield 150

    start(("q", 0))
    start(("w1", 0))
    for g in range(G):
        k_buf[g, pl.ds(0, 8), :] = jnp.zeros((8, 128), u32)
    b1_buf[...] = b1_ref[...].astype(f32).reshape(1, F)
    bt_buf[...] = jnp.broadcast_to(b1_buf[:, F - F % 128:], (128, F % 128)).T
    b2_buf[...] = b2_ref[...].astype(f32).reshape(1, D)
    with _scope("M0"):
        wait(("q", 0))
        start(("q", 1))
        start(("w1", 1))
        _Fill(norm(0))(ALL)
        wait(("w1", 0))
        mm1(0, _Fill(()), 0, WCH[0], WCH[1])
        wait(("q", 1))
        start(("w1", 2), ("q", 2))
        _Fill(norm(1))(ALL)
        mm1(1, _Fill(()), 0, WCH[0], WCH[1])
        wait(("w1", 1))
        start(W2)
        for i in range(2):
            mm1(i, _Fill(()), 0, WCH[1], WCH[2])
        wait(("w1", 2))
        wait(("q", 2))
        start(("q", 3))
        fill = _Fill(norm(2, 3))
        for i in range(2):
            mm1(i, fill, FILLM, WCH[2], WCH[3])
        fill(ALL)
        start(("q", 4))
        wait(W2)
        wait(("q", 3))
        start(FWD, *conv_in(0, 1, 2))

    with _scope("A"):
        @pl.loop(0, 2)
        def _(i):
            @pl.when(i == 1)
            def _():
                wait(("q", 4))
                start(*conv_in(3, 4))

            fill = _Fill(norm(4 + i))
            mm2(i, fill, 40)
            fill(ALL)
            mm1(i + 2, fill, 0)

    wait(FWD, *conv_in(0, 1, 2))
    start(INV)
    with _scope("prep0"):
        _Fill(prep(0))(ALL)
    with _scope("B"):
        for g in range(G - 1):
            if g == 2:
                wait(*conv_in(3, 4))
            stage1(g, prep(g + 1))

    with _scope("S4"):
        stage1(G - 1, norm(6, 7, cost=450))

    with _scope("C"):
        @pl.loop(0, G - 1)
        def _(g):
            fill = _Fill(middle(g * NU, NU))
            mm2(g + 2, fill, FILL2)
            mm1(g + 4, fill, FILL1)
            fill(ALL)

    wait(INV)
    with _scope("I"):
        if UNI:
            for g in range(G):
                inverse(g)
        else:
            pl.loop(0, G)(inverse)

    with _scope("E"):
        fill = _Fill(final([i for i in range(NB - 2)]))
        mm2(NB - 2, fill, FILLE, last=True)
        fill(ALL)

        out_copy(0).start()
        mm2(NB - 1, _Fill(()), 0, last=True)
        out_copy(1).start()
    out_copy(0).wait()
    out_copy(1).wait()


OCH = (0, NB - 1, NB)
FILL1, FILL2 = 350, 115
ALL = 10**9
WCH = (0, 256, 768, F)
QCH = (0, 1, 2, 4, 5, NB)
W2, FWD, INV = ("mat", 0), ("mat", 1), ("mat", 2)
COPIES = ([("q", i) for i in range(5)] + [("w1", i) for i in range(3)] + [W2, FWD, INV]
          + [(kind, g) for g in range(G) for kind in ("ssm", "k", "v")])
NU = G * (N1 // 8) // 4
YY = N1 + 1
YP = N1 + 32


def _yrow(src, n, part):
    return ((src * N2 + n) * 2 + part) * YP + 8 * ((n // 4 + 2 * part) % 4)


NF = (F + 127) // 128
KH = 512
LC = 32
KP = 17


FILLB, FILLE, FILLM = 225, 70, 250
UNI = 1


def _words(m):
    u = np.ascontiguousarray(m).view(np.uint16).astype(np.uint32)
    return u[..., 0::2, :] | (u[..., 1::2, :] << 16)


def _perm_fwd():
    r = np.arange(N1)
    n1 = r // 2 + (N1 // 2) * (r % 2)
    return _words(_FWD[:, :, n1])


_FWD_P = _perm_fwd()
_INV_P = _words(_INV)


@jax.jit
def pallas_parallel_sum__ssm_conv_h3__dense_activation_gelu__prompt_kernel(
    A_q, A_k, A_v, A_shift_k, A_ssm_k, A_ssm_D, B_x, B_w1, B_b1, B_w2, B_b2,
):
    hbm = pl.BlockSpec(memory_space=pl.ANY)
    vmem = pl.BlockSpec(memory_space=pltpu.VMEM)
    return pl.pallas_call(
        _kernel,
        out_shape=jax.ShapeDtypeStruct((1, S, D), bf16),
        in_specs=[hbm, hbm, hbm, vmem, hbm, vmem, hbm, vmem, hbm, vmem, hbm, hbm,
                  pl.BlockSpec(memory_space=pltpu.SMEM)],
        out_specs=hbm,
        scratch_shapes=[
            pltpu.VMEM((S // 2, D), u32),
            pltpu.VMEM((G, S // 2 + 16, 128), u32),
            pltpu.VMEM((G, S // 2 + 8, 128), u32),
            pltpu.VMEM((D // 2, S), u32),
            pltpu.VMEM((F // 2, D), u32),
            pltpu.VMEM((F // 2, D), u32),
            pltpu.VMEM((N2, N1, N1), u32),
            pltpu.VMEM((N2, N1 // 2, N1), u32),
            pltpu.VMEM((G, KP * (N1 // 2 + 1), 128), u32),
            pltpu.VMEM((G, N2, N1 // 2, 128), u32),
            pltpu.VMEM((G, 9 * YY, 128), u32),
            pltpu.VMEM((S // 2, D), u32),
            pltpu.VMEM((S // 2, F), u32),
            pltpu.VMEM((G, S, 128), f32),
            pltpu.VMEM((G, 6 * N2 * YP, 128), f32),
            pltpu.VMEM((1, F), f32),
            pltpu.VMEM((F % 128, 128), f32),
            pltpu.VMEM((1, D), f32),
            pltpu.SemaphoreType.DMA((len(COPIES),)),
            pltpu.SemaphoreType.DMA((2,)),
        ],
        compiler_params=pltpu.CompilerParams(vmem_limit_bytes=100 * 2**20),
    )(A_q, A_k, A_v, A_shift_k.T, A_ssm_k,
      A_ssm_D, B_w1.T, B_b1, B_w2, B_b2, _FWD_P, _INV_P, np.zeros((1,), np.int32))
```

```python
import contextlib

import jax
import jax.numpy as jnp
import numpy as np
import jax.experimental.pallas as pl
import jax.experimental.pallas.tpu as pltpu

S, D, F, KS = 2048, 640, 1728, 4
N1, N2 = 128, 16
G = D // 128
BM = 256
NB = S // BM
bf16, f32, u32 = jnp.bfloat16, jnp.float32, jnp.uint32


def _dft_mats():
    k1 = np.arange(N1)[None, :, None]
    n1 = np.arange(N1)[None, None, :]
    n2 = np.arange(N2)[:, None, None]
    ang = -2.0 * np.pi * (k1 + 0.25) * (N2 * n1 + n2) / S
    fr, fi = np.cos(ang), np.sin(ang)
    fwd = np.concatenate([fr, fi], axis=1)
    inv = np.concatenate([fr[:, :N1 // 2], fi[:, :N1 // 2]], axis=1)
    inv = np.transpose(inv, (0, 2, 1)) / S
    inv = np.concatenate([inv[:, 0::2], inv[:, 1::2]], axis=1)
    return fwd.astype(jnp.bfloat16), inv.astype(jnp.bfloat16)


_FWD, _INV = _dft_mats()

_C1, _S1, _R2 = float(np.cos(np.pi / 8)), float(np.sin(np.pi / 8)), float(np.sqrt(0.5))


def _bf4(a, b, c, d, sgn):
    t0 = (a[0] + c[0], a[1] + c[1])
    t1 = (a[0] - c[0], a[1] - c[1])
    t2 = (b[0] + d[0], b[1] + d[1])
    t3 = (b[0] - d[0], b[1] - d[1])
    o0 = (t0[0] + t2[0], t0[1] + t2[1])
    o2 = (t0[0] - t2[0], t0[1] - t2[1])
    p = (t1[0] + t3[1], t1[1] - t3[0])
    q = (t1[0] - t3[1], t1[1] + t3[0])
    return (o0, p, o2, q) if sgn < 0 else (o0, q, o2, p)


def _tw(x, e, sgn):
    r, i = x
    if e == 0:
        return x
    if e == 4:
        return (i, -r) if sgn < 0 else (-i, r)
    if e == 2:
        return ((r + i) * _R2, (i - r) * _R2) if sgn < 0 else ((r - i) * _R2, (r + i) * _R2)
    if e == 6:
        return ((i - r) * _R2, (r + i) * -_R2) if sgn < 0 else ((r + i) * -_R2, (r - i) * _R2)
    c = float(np.cos(2 * np.pi * e / 16))
    s = sgn * float(np.sin(2 * np.pi * e / 16))
    return (r * c - i * s, r * s + i * c)


_TWC = (16, 32, 24, 32)


def _lo(w):
    return pltpu.bitcast(w << 16, f32)


def _hi(w):
    return pltpu.bitcast(w & u32(0xFFFF0000), f32)


def _pack(a, b):
    return jnp.concatenate([a, b], axis=0).astype(bf16)


def _gelu(h):
    c1 = 0.7978845608028654
    u = h * (c1 + (c1 * 0.044715) * (h * h))
    hh = 0.5 * h
    return hh + hh * jnp.tanh(u)


def _scope(name):
    return contextlib.nullcontext()


class _Fill:
    def __init__(self, steps):
        self.it = iter(steps)
        self.debt = 0

    def __call__(self, budget):
        self.debt += budget
        while self.debt > 0:
            c = next(self.it, None)
            if c is None:
                return
            self.debt -= c


def _kernel(q_hbm, k_hbm, v_hbm, sk_ref, ssm_hbm, d_ref, w1_hbm, b1_ref, w2_hbm, b2_ref,
            fwd_hbm, inv_hbm, zero_ref, o_hbm,
            q_buf, k_buf, v_buf, ssm_buf, w1_buf, w2_buf, fwd_buf, inv_buf,
            kt_buf, rhs_buf, y_buf, xn_buf, h_buf, acc, fb, b1_buf, bt_buf, b2_buf, sems, osems):
    qw, kw, vw, sw, w1w, w2w = (r.bitcast(u32) for r in (q_hbm, k_hbm, v_hbm, ssm_hbm, w1_hbm, w2_hbm))
    HB = BM // 2
    z0 = zero_ref[0]

    def copy(name):
        kind, i = name
        if kind == "q":
            rs = pl.ds(QCH[i] * HB, (QCH[i + 1] - QCH[i]) * HB)
            src, dst = qw.at[0, rs], q_buf.at[rs]
        elif kind == "w1":
            rs = pl.ds(WCH[i] // 2, (WCH[i + 1] - WCH[i]) // 2)
            src, dst = w1w.at[rs], w1_buf.at[rs]
        elif kind == "ssm":
            src, dst = sw.at[rows(i, 64)], ssm_buf.at[rows(i, 64)]
        elif kind == "k":
            src, dst = kw.at[0, :, rows(i, 128)], k_buf.at[i, pl.ds(8, S // 2)]
        elif kind == "v":
            src, dst = vw.at[0, :, rows(i, 128)], v_buf.at[i, pl.ds(0, S // 2)]
        else:
            src, dst = ((w2w, w2_buf), (fwd_hbm, fwd_buf), (inv_hbm, inv_buf))[i]
        return pltpu.make_async_copy(src, dst, sems.at[COPIES.index(name)])

    def start(*names):
        for name in names:
            copy(name).start()

    def wait(*names):
        for name in names:
            copy(name).wait()

    def conv_in(*groups):
        return [(kind, g) for g in groups for kind in ("ssm", "k", "v")]

    def rows(i, n):
        return pl.ds(i * n if isinstance(i, int) else pl.multiple_of(i * n, n), n)

    def norm(*blocks):
        for i in blocks:
            for c in range(BM // LC):
                x = pltpu.bitcast(q_buf[rows(i * (BM // LC) + c, LC // 2), :], bf16).astype(f32)
                m = jnp.mean(x, axis=-1, keepdims=True)
                xc = x - m
                var = jnp.mean(xc * xc, axis=-1, keepdims=True)
                xn = (xc * jax.lax.rsqrt(var + 1e-5)).astype(bf16)
                xn_buf[rows(i * (BM // LC) + c, LC // 2), :] = pltpu.bitcast(xn, u32)
                yield LC * 6

    def mm1(i, fill, cost, lo=0, hi=F):
        for f0 in range(lo, hi, 128):
            f1 = min(F, f0 + 128)
            xn = pltpu.bitcast(xn_buf[rows(i, HB), :], bf16)
            w = pltpu.bitcast(w1_buf[f0 // 2:f1 // 2, :], bf16)
            nt = (((1,), (1,)), ((), ()))
            if f1 - f0 == 128:
                h = jax.lax.dot_general(xn, w, nt, preferred_element_type=f32)
                h = _gelu(h + b1_buf[:, f0:f1])
            else:
                h = jax.lax.dot_general(w, xn, nt, preferred_element_type=f32)
                h = _gelu(h + jnp.tile(bt_buf[...], (1, BM // 128))).T
            h_buf[rows(i, HB), f0:f1] = pltpu.bitcast(h.astype(bf16), u32)
            fill(cost)

    def mm2(i, fill, cost, last=False):
        for g in range(G):
            ls = slice(g * 128, (g + 1) * 128)
            for f0 in range(0, F, KH):
                f1 = min(F, f0 + KH)
                h = pltpu.bitcast(h_buf[rows(i, HB), f0:f1], bf16)
                p = jnp.dot(h, pltpu.bitcast(w2_buf[f0 // 2:f1 // 2, ls], bf16),
                            preferred_element_type=f32)
                if last:
                    c = f0 // KH
                    if c:
                        p = acc[g, rows(i + z0, BM), :] + p
                    x = pltpu.bitcast(q_buf[rows(4 * (i + z0) + c, HB // 4), ls], bf16).astype(f32)
                    o = [p[r:r + BM // 4] for r in range(0, BM, BM // 4)]
                    o[c] = o[c] + (x + b2_buf[:, ls])
                    o = jnp.concatenate(o, axis=0)
                elif f0 == 0:
                    x = pltpu.bitcast(q_buf[rows(i, HB), ls], bf16).astype(f32)
                    o = p + (x + b2_buf[:, ls])
                else:
                    o = o + p
                if last and f1 == F:
                    gate(i, g, o)
                elif last or f1 == F:
                    acc[g, rows(i, BM), :] = o
                fill(cost * (f1 - f0) // 128)

    def prep(g):
        if g >= 0:
            sk = sk_ref[:, g * 128:(g + 1) * 128].astype(f32)
            sk = [jnp.broadcast_to(sk[j:j + 1, :], (8, 128)) for j in range(KS)]
        for a in range(8):
            if g + 1 < G:
                for c in (2 * a, 2 * a + 1):
                    kt = pltpu.bitcast(ssm_buf[rows(g + 1, 64), rows(c, 128)], bf16).astype(f32).T
                    if c == 0:
                        dd = d_ref[...].astype(f32).reshape(1, D)[:, (g + 1) * 128:(g + 2) * 128]
                        row = jax.lax.broadcasted_iota(jnp.int32, (N2, 128), 0)
                        top = kt[:N2] + jnp.where(row == 0, jnp.broadcast_to(dd, (N2, 128)), 0.0)
                        kt = jnp.concatenate([top.astype(bf16).astype(f32), kt[N2:]], axis=0)
                    kt = pltpu.bitcast(kt, u32)
                    for j in range(4):
                        r = 2 * N2 * j
                        kt_buf[g + 1, pl.ds(KP * (4 * c + j), N2), :] = (
                            (kt[r:r + N2] >> 16) | kt[r + N2:r + 2 * N2])
                yield 96
            if g < 0:
                continue
            res = []
            for hf in range(2):
                base = a * 128 + hf * 64
                w = [kw_ld(g, base + 8 + m) for m in range(-2, 8)]
                ks = [f(x) for x in w for f in (_lo, _hi)]
                kv = []
                for m in range(8):
                    w = v_buf[g, pl.ds(base + m, 8, stride=8), :]
                    for p, vv in enumerate((_lo(w), _hi(w))):
                        n = 4 + 2 * m + p
                        s = (ks[n] * sk[0] + ks[n - 1] * sk[1]) + (ks[n - 2] * sk[2] + ks[n - 3] * sk[3])
                        kv.append(s * vv)
                res.append(kv)
                yield 172
            for n in range(N2):
                rhs_buf[g, n, pl.ds(a * 8, 8), :] = pltpu.bitcast(_pack(res[0][n], res[1][n]), u32)

    def kw_ld(g, r):
        return k_buf[g, pl.ds(r, 8, stride=8), :]

    def stage1(g, side, cost):
        fill = _Fill(side)
        for n in range(N2):
            ops = []
            if g >= 0:
                ops.append((0, g, pltpu.bitcast(rhs_buf[g, n], bf16)))
            if g + 1 < G:
                kk = kt_buf[g + 1, pl.ds(n, N1 // 2, stride=KP), :]
                ops.append((1, g + 1, pltpu.bitcast(kk, bf16)))
            rhs = jnp.concatenate([op[2] for op in ops], axis=1)
            y = jnp.dot(pltpu.bitcast(fwd_buf[n], bf16), rhs, preferred_element_type=f32)
            for j, (src, gg, _) in enumerate(ops):
                for part in range(2):
                    fb[gg, pl.ds(_yrow(src, n, part), N1), :] = (
                        y[part * N1:(part + 1) * N1, j * 128:(j + 1) * 128])
            fill(cost)
        fill(ALL)

    def spectrum_product(g, a):
        ys = []
        for src in (1, 0):
            y = [[None] * 4 for _ in range(4)]
            for b in range(4):
                x = [tuple(fb[g, pl.ds(a + _yrow(src, n, part), 8), :] for part in range(2))
                     for n in range(b, N2, 4)]
                o = _bf4(*x, -1)
                for c in range(4):
                    y[c][b] = _tw(o[c], b * c, -1)
                yield _TWC[b]
            ys.append(y)
        w = [[None] * 4 for _ in range(4)]
        for c in range(4):
            sb = _bf4(*ys[0][c], -1)
            sa = _bf4(*ys[1][c], -1)
            pr = [(p[0] * q[0] - p[1] * q[1], p[0] * q[1] + p[1] * q[0]) for p, q in zip(sa, sb)]
            o = _bf4(*pr, 1)
            for e in range(4):
                w[e][c] = _tw(o[e], c * e, 1)
            yield 56 + _TWC[c]
        return w

    def middle(u0, nu):
        for u in range(nu):
            g = (u0 + u) // (N1 // 8)
            a = pl.multiple_of((u0 + u) % (N1 // 8) * 8, 8)
            w = yield from spectrum_product(g, a)
            for e in range(4):
                o = _bf4(*w[e], 1)
                for d in range(4):
                    for part in range(2):
                        fb[g, pl.ds(a + _yrow(2, e + 4 * d, part), 8), :] = o[d][part]
                yield 20

    def inverse(g):
        H = N1 // 2
        for n in range(N2):
            lo, hi = (tuple(fb[g, pl.ds(_yrow(2, n, part) + r, H), :] for part in range(2))
                      for r in (0, H))
            t = _tw(hi, n / 2, 1)
            zs = (_pack(lo[0] + t[0], lo[1] + t[1]), _pack(lo[0] - t[0], lo[1] - t[1]))
            for par in range(2):
                y_buf[g, pl.ds(n * YY + par * H, H), :] = jnp.dot(
                    pltpu.bitcast(inv_buf[n, rows(par, H // 2), :], bf16), zs[par],
                    preferred_element_type=f32)

    def out_copy(j):
        rs = pl.ds(OCH[j] * HB, (OCH[j + 1] - OCH[j]) * HB)
        return pltpu.make_async_copy(q_buf.at[rs], o_hbm.bitcast(u32).at[0, rs], osems.at[j])

    def gate(i, g, o):
        y = jnp.concatenate(
            [y_buf[g, pl.ds(i * (BM // 32) + (n // 2 + n % 2 * (N1 // 2) + h * YY), 8, stride=YY), :]
             for n in range(BM // N2) for h in (0, 8)], axis=0)
        xn = pltpu.bitcast(xn_buf[rows(i, HB), rows(g, 128)], bf16).astype(f32)
        q_buf[rows(i, HB), rows(g, 128)] = pltpu.bitcast((o + xn * y).astype(bf16), u32)

    def final(blocks):
        for i in blocks:
            for g in range(G):
                gate(i, g, acc[g, rows(i, BM), :])
                yield 150

    start(("q", 0))
    start(("w1", 0))
    for g in range(G):
        k_buf[g, pl.ds(0, 8), :] = jnp.zeros((8, 128), u32)
    b1_buf[...] = b1_ref[...].astype(f32).reshape(1, F)
    bt_buf[...] = jnp.broadcast_to(b1_buf[:, F - F % 128:], (128, F % 128)).T
    b2_buf[...] = b2_ref[...].astype(f32).reshape(1, D)
    with _scope("M0"):
        wait(("q", 0))
        start(("q", 1))
        start(("w1", 1))
        _Fill(norm(0))(ALL)
        wait(("w1", 0))
        mm1(0, _Fill(()), 0, WCH[0], WCH[1])
        wait(("q", 1))
        start(("w1", 2), ("q", 2))
        _Fill(norm(1))(ALL)
        mm1(1, _Fill(()), 0, WCH[0], WCH[1])
        wait(("w1", 1))
        start(W2)
        for i in range(2):
            mm1(i, _Fill(()), 0, WCH[1], WCH[2])
        wait(("w1", 2))
        wait(("q", 2))
        start(("q", 3))
        fill = _Fill(norm(2, 3))
        for i in range(2):
            mm1(i, fill, FILLM, WCH[2], WCH[3])
        fill(ALL)
        start(("q", 4))
        wait(W2)
        wait(("q", 3))
        start(FWD, *conv_in(0, 1, 2))

    with _scope("A"):
        @pl.loop(0, 2)
        def _(i):
            @pl.when(i == 1)
            def _():
                wait(("q", 4))
                start(*conv_in(3, 4))

            fill = _Fill(norm(4 + i))
            mm2(i, fill, 40)
            fill(ALL)
            mm1(i + 2, fill, 0)

    wait(FWD, *conv_in(0, 1, 2))
    start(INV)
    with _scope("B"):
        _Fill(prep(-1))(ALL)
        for g in range(-1, G):
            if g == 1:
                wait(*conv_in(3, 4))
            stage1(g, prep(g + 1) if g + 1 < G else norm(6, 7), FILLB)

    with _scope("C"):
        @pl.loop(0, G - 1)
        def _(g):
            fill = _Fill(middle(g * NU, NU))
            mm2(g + 2, fill, FILL2)
            mm1(g + 4, fill, FILL1)
            fill(ALL)

    wait(INV)
    with _scope("I"):
        if UNI:
            for g in range(G):
                inverse(g)
        else:
            pl.loop(0, G)(inverse)

    with _scope("E"):
        fill = _Fill(final([i for i in range(NB - 2)]))
        mm2(NB - 2, fill, FILLE, last=True)
        fill(ALL)

        out_copy(0).start()
        mm2(NB - 1, _Fill(()), 0, last=True)
        out_copy(1).start()
    out_copy(0).wait()
    out_copy(1).wait()


OCH = (0, NB - 1, NB)
FILL1, FILL2 = 350, 115
ALL = 10**9
WCH = (0, 256, 768, F)
QCH = (0, 1, 2, 4, 5, NB)
W2, FWD, INV = ("mat", 0), ("mat", 1), ("mat", 2)
COPIES = ([("q", i) for i in range(5)] + [("w1", i) for i in range(3)] + [W2, FWD, INV]
          + [(kind, g) for g in range(G) for kind in ("ssm", "k", "v")])
NU = G * (N1 // 8) // 4
YY = N1 + 1
YP = N1 + 32


def _yrow(src, n, part):
    return ((src * N2 + n) * 2 + part) * YP + 8 * ((n // 4 + 2 * part) % 4)


NF = (F + 127) // 128
KH = 512
LC = 32
KP = 17


FILLB, FILLE, FILLM = 225, 70, 250
UNI = 1
P1, P2, P3 = 24, 0, 0


def _words(m):
    u = np.ascontiguousarray(m).view(np.uint16).astype(np.uint32)
    return u[..., 0::2, :] | (u[..., 1::2, :] << 16)


_FWD_P = _words(_FWD)
_INV_P = _words(_INV)


@jax.jit
def pallas_parallel_sum__ssm_conv_h3__dense_activation_gelu__prompt_kernel(
    A_q, A_k, A_v, A_shift_k, A_ssm_k, A_ssm_D, B_x, B_w1, B_b1, B_w2, B_b2,
):
    hbm = pl.BlockSpec(memory_space=pl.ANY)
    vmem = pl.BlockSpec(memory_space=pltpu.VMEM)
    return pl.pallas_call(
        _kernel,
        out_shape=jax.ShapeDtypeStruct((1, S, D), bf16),
        in_specs=[hbm, hbm, hbm, vmem, hbm, vmem, hbm, vmem, hbm, vmem, hbm, hbm,
                  pl.BlockSpec(memory_space=pltpu.SMEM)],
        out_specs=hbm,
        scratch_shapes=[
            pltpu.VMEM((S // 2, D), u32),
            pltpu.VMEM((G, S // 2 + 16, 128), u32),
            pltpu.VMEM((G, S // 2 + 8, 128), u32),
            pltpu.VMEM((D // 2, S), u32),
            pltpu.VMEM((F // 2, D), u32),
            pltpu.VMEM((F // 2, D), u32),
            pltpu.VMEM((N2, N1, N1), u32),
            pltpu.VMEM((N2, N1 // 2, N1), u32),
            pltpu.VMEM((G, KP * (N1 // 2 + 1), 128), u32),
            pltpu.VMEM((G, N2, N1 // 2, 128), u32),
            pltpu.VMEM((G, (N2 + 1) * YY + P1, 128), f32),
            pltpu.VMEM((S // 2 + P3, D), u32),
            pltpu.VMEM((S // 2, F), u32),
            pltpu.VMEM((G, S + P2, 128), f32),
            pltpu.VMEM((G, 6 * N2 * YP, 128), f32),
            pltpu.VMEM((1, F), f32),
            pltpu.VMEM((F % 128, 128), f32),
            pltpu.VMEM((1, D), f32),
            pltpu.SemaphoreType.DMA((len(COPIES),)),
            pltpu.SemaphoreType.DMA((2,)),
        ],
        compiler_params=pltpu.CompilerParams(vmem_limit_bytes=100 * 2**20),
    )(A_q, A_k, A_v, A_shift_k.T, A_ssm_k,
      A_ssm_D, B_w1.T, B_b1, B_w2, B_b2, _FWD_P, _INV_P, np.zeros((1,), np.int32))
```

```python
import jax
import jax.numpy as jnp
import numpy as np
import jax.experimental.pallas as pl
import jax.experimental.pallas.tpu as pltpu

S, D, F, KS = 2048, 640, 1728, 4
N1, N2 = 128, 16
G = D // 128
BM = 256
NB = S // BM
bf16, f32, u32 = jnp.bfloat16, jnp.float32, jnp.uint32


def _dft_mats():
    k1 = np.arange(N1)[None, :, None]
    n1 = np.arange(N1)[None, None, :]
    n2 = np.arange(N2)[:, None, None]
    ang = -2.0 * np.pi * (k1 + 0.25) * (N2 * n1 + n2) / S
    fr, fi = np.cos(ang), np.sin(ang)
    fwd = np.concatenate([fr, fi], axis=1)
    inv = np.concatenate([fr[:, :N1 // 2], fi[:, :N1 // 2]], axis=1)
    inv = np.transpose(inv, (0, 2, 1)) / S
    inv = np.concatenate([inv[:, 0::2], inv[:, 1::2]], axis=1)
    return fwd.astype(jnp.bfloat16), inv.astype(jnp.bfloat16)


_FWD, _INV = _dft_mats()

_R2 = float(np.sqrt(0.5))


def _bf4(a, b, c, d, sgn):
    t0 = (a[0] + c[0], a[1] + c[1])
    t1 = (a[0] - c[0], a[1] - c[1])
    t2 = (b[0] + d[0], b[1] + d[1])
    t3 = (b[0] - d[0], b[1] - d[1])
    o0 = (t0[0] + t2[0], t0[1] + t2[1])
    o2 = (t0[0] - t2[0], t0[1] - t2[1])
    p = (t1[0] + t3[1], t1[1] - t3[0])
    q = (t1[0] - t3[1], t1[1] + t3[0])
    return (o0, p, o2, q) if sgn < 0 else (o0, q, o2, p)


def _tw(x, e, sgn):
    r, i = x
    if e == 0:
        return x
    if e == 4:
        return (i, -r) if sgn < 0 else (-i, r)
    if e == 2:
        return ((r + i) * _R2, (i - r) * _R2) if sgn < 0 else ((r - i) * _R2, (r + i) * _R2)
    if e == 6:
        return ((i - r) * _R2, (r + i) * -_R2) if sgn < 0 else ((r + i) * -_R2, (r - i) * _R2)
    c = float(np.cos(2 * np.pi * e / 16))
    s = sgn * float(np.sin(2 * np.pi * e / 16))
    return (r * c - i * s, r * s + i * c)


_TWC = (16, 32, 24, 32)


def _lo(w):
    return pltpu.bitcast(w << 16, f32)


def _hi(w):
    return pltpu.bitcast(w & np.uint32(0xFFFF0000), f32)


def _pack(a, b):
    return jnp.concatenate([a, b], axis=0).astype(bf16)


def _gelu(h):
    c1 = 0.7978845608028654
    u = h * (c1 + (c1 * 0.044715) * (h * h))
    hh = 0.5 * h
    return hh + hh * jnp.tanh(u)


class _Fill:
    def __init__(self, steps):
        self.it = iter(steps)
        self.debt = 0

    def __call__(self, budget):
        self.debt += budget
        while self.debt > 0:
            c = next(self.it, None)
            if c is None:
                return
            self.debt -= c


def _kernel(q_hbm, k_hbm, v_hbm, sk_ref, ssm_hbm, d_ref, w1_hbm, b1_ref, w2_hbm, b2_ref,
            fwd_hbm, inv_hbm, zero_ref, o_hbm,
            q_buf, k_buf, v_buf, ssm_buf, w1_buf, w2_buf, fwd_buf, inv_buf,
            kt_buf, rhs_buf, y_buf, xn_buf, h_buf, acc, fb, b1_buf, bt_buf, b2_buf, sems, osems):
    qw, kw, vw, sw, w1w, w2w = (r.bitcast(u32) for r in (q_hbm, k_hbm, v_hbm, ssm_hbm, w1_hbm, w2_hbm))
    HB = BM // 2
    z0 = zero_ref[0]

    def copy(name):
        kind, i = name
        if kind == "q":
            rs = pl.ds(QCH[i] * HB, (QCH[i + 1] - QCH[i]) * HB)
            src, dst = qw.at[0, rs], q_buf.at[rs]
        elif kind == "w1":
            rs = pl.ds(WCH[i] // 2, (WCH[i + 1] - WCH[i]) // 2)
            src, dst = w1w.at[rs], w1_buf.at[rs]
        elif kind == "ssm":
            src, dst = sw.at[rows(i, 64)], ssm_buf.at[rows(i, 64)]
        elif kind == "k":
            src, dst = kw.at[0, :, rows(i, 128)], k_buf.at[i, pl.ds(8, S // 2)]
        elif kind == "v":
            src, dst = vw.at[0, :, rows(i, 128)], v_buf.at[i, pl.ds(0, S // 2)]
        else:
            src, dst = ((w2w, w2_buf), (fwd_hbm, fwd_buf), (inv_hbm, inv_buf))[i]
        return pltpu.make_async_copy(src, dst, sems.at[COPIES.index(name)])

    def start(*names):
        for name in names:
            copy(name).start()

    def wait(*names):
        for name in names:
            copy(name).wait()

    def conv_in(*groups):
        return [(kind, g) for g in groups for kind in ("ssm", "k", "v")]

    def rows(i, n):
        return pl.ds(i * n if isinstance(i, int) else pl.multiple_of(i * n, n), n)

    def norm(*blocks):
        for i in blocks:
            for c in range(BM // LC):
                x = pltpu.bitcast(q_buf[rows(i * (BM // LC) + c, LC // 2), :], bf16).astype(f32)
                m = jnp.mean(x, axis=-1, keepdims=True)
                xc = x - m
                var = jnp.mean(xc * xc, axis=-1, keepdims=True)
                xn = (xc * jax.lax.rsqrt(var + 1e-5)).astype(bf16)
                xn_buf[rows(i * (BM // LC) + c, LC // 2), :] = pltpu.bitcast(xn, u32)
                yield LC * 6

    def mm1(i, fill, cost, lo=0, hi=F):
        for f0 in range(lo, hi, 128):
            f1 = min(F, f0 + 128)
            xn = pltpu.bitcast(xn_buf[rows(i, HB), :], bf16)
            w = pltpu.bitcast(w1_buf[f0 // 2:f1 // 2, :], bf16)
            nt = (((1,), (1,)), ((), ()))
            if f1 - f0 == 128:
                h = jax.lax.dot_general(xn, w, nt, preferred_element_type=f32)
                h = _gelu(h + b1_buf[:, f0:f1])
            else:
                h = jax.lax.dot_general(w, xn, nt, preferred_element_type=f32)
                h = _gelu(h + jnp.tile(bt_buf[...], (1, BM // 128))).T
            h_buf[rows(i, HB), f0:f1] = pltpu.bitcast(h.astype(bf16), u32)
            fill(cost)

    def mm2(i, fill, cost, last=False):
        for g in range(G):
            ls = slice(g * 128, (g + 1) * 128)
            for f0 in range(0, F, KH):
                f1 = min(F, f0 + KH)
                h = pltpu.bitcast(h_buf[rows(i, HB), f0:f1], bf16)
                p = jnp.dot(h, pltpu.bitcast(w2_buf[f0 // 2:f1 // 2, ls], bf16),
                            preferred_element_type=f32)
                if last:
                    c = f0 // KH
                    if c:
                        p = acc[g, rows(i + z0, BM), :] + p
                    x = pltpu.bitcast(q_buf[rows(4 * (i + z0) + c, HB // 4), ls], bf16).astype(f32)
                    o = [p[r:r + BM // 4] for r in range(0, BM, BM // 4)]
                    o[c] = o[c] + (x + b2_buf[:, ls])
                    o = jnp.concatenate(o, axis=0)
                elif f0 == 0:
                    x = pltpu.bitcast(q_buf[rows(i, HB), ls], bf16).astype(f32)
                    o = p + (x + b2_buf[:, ls])
                else:
                    o = o + p
                if last and f1 == F:
                    gate(i, g, o)
                elif last or f1 == F:
                    acc[g, rows(i, BM), :] = o
                fill(cost * (f1 - f0) // 128)

    def prep(g):
        if g >= 0:
            sk = sk_ref[:, g * 128:(g + 1) * 128].astype(f32)
            sk = [jnp.broadcast_to(sk[j:j + 1, :], (8, 128)) for j in range(KS)]
        for a in range(8):
            if g + 1 < G:
                for c in (2 * a, 2 * a + 1):
                    kt = pltpu.bitcast(ssm_buf[rows(g + 1, 64), rows(c, 128)], bf16).astype(f32).T
                    if c == 0:
                        dd = d_ref[...].astype(f32).reshape(1, D)[:, (g + 1) * 128:(g + 2) * 128]
                        row = jax.lax.broadcasted_iota(jnp.int32, (N2, 128), 0)
                        top = kt[:N2] + jnp.where(row == 0, jnp.broadcast_to(dd, (N2, 128)), 0.0)
                        kt = jnp.concatenate([top.astype(bf16).astype(f32), kt[N2:]], axis=0)
                    kt = pltpu.bitcast(kt, u32)
                    for j in range(4):
                        r = 2 * N2 * j
                        kt_buf[g + 1, pl.ds(KP * (4 * c + j), N2), :] = (
                            (kt[r:r + N2] >> 16) | kt[r + N2:r + 2 * N2])
                yield 96
            if g < 0:
                continue
            res = []
            for hf in range(2):
                base = a * 128 + hf * 64
                w = [kw_ld(g, base + 8 + m) for m in range(-2, 8)]
                ks = [f(x) for x in w for f in (_lo, _hi)]
                kv = []
                for m in range(8):
                    w = v_buf[g, pl.ds(base + m, 8, stride=8), :]
                    for p, vv in enumerate((_lo(w), _hi(w))):
                        n = 4 + 2 * m + p
                        s = (ks[n] * sk[0] + ks[n - 1] * sk[1]) + (ks[n - 2] * sk[2] + ks[n - 3] * sk[3])
                        kv.append(s * vv)
                res.append(kv)
                yield 172
            for n in range(N2):
                rhs_buf[g, n, pl.ds(a * 8, 8), :] = pltpu.bitcast(_pack(res[0][n], res[1][n]), u32)

    def kw_ld(g, r):
        return k_buf[g, pl.ds(r, 8, stride=8), :]

    def stage1(g, side, cost):
        fill = _Fill(side)
        for n in range(N2):
            ops = []
            if g >= 0:
                ops.append((0, g, pltpu.bitcast(rhs_buf[g, n], bf16)))
            if g + 1 < G:
                kk = kt_buf[g + 1, pl.ds(n, N1 // 2, stride=KP), :]
                ops.append((1, g + 1, pltpu.bitcast(kk, bf16)))
            rhs = jnp.concatenate([op[2] for op in ops], axis=1)
            y = jnp.dot(pltpu.bitcast(fwd_buf[n], bf16), rhs, preferred_element_type=f32)
            for j, (src, gg, _) in enumerate(ops):
                for part in range(2):
                    fb[gg, pl.ds(_yrow(src, n, part), N1), :] = (
                        y[part * N1:(part + 1) * N1, j * 128:(j + 1) * 128])
            fill(cost)
        fill(ALL)

    def spectrum_product(g, a):
        ys = []
        for src in (1, 0):
            y = [[None] * 4 for _ in range(4)]
            for b in range(4):
                x = [tuple(fb[g, pl.ds(a + _yrow(src, n, part), 8), :] for part in range(2))
                     for n in range(b, N2, 4)]
                o = _bf4(*x, -1)
                for c in range(4):
                    y[c][b] = _tw(o[c], b * c, -1)
                yield _TWC[b]
            ys.append(y)
        w = [[None] * 4 for _ in range(4)]
        for c in range(4):
            sb = _bf4(*ys[0][c], -1)
            sa = _bf4(*ys[1][c], -1)
            pr = [(p[0] * q[0] - p[1] * q[1], p[0] * q[1] + p[1] * q[0]) for p, q in zip(sa, sb)]
            o = _bf4(*pr, 1)
            for e in range(4):
                w[e][c] = _tw(o[e], c * e, 1)
            yield 56 + _TWC[c]
        return w

    def middle(u0, nu):
        for u in range(nu):
            g = (u0 + u) // (N1 // 8)
            a = pl.multiple_of((u0 + u) % (N1 // 8) * 8, 8)
            w = yield from spectrum_product(g, a)
            for e in range(4):
                o = _bf4(*w[e], 1)
                for d in range(4):
                    for part in range(2):
                        fb[g, pl.ds(a + _yrow(2, e + 4 * d, part), 8), :] = o[d][part]
                yield 20

    def inverse(g):
        H = N1 // 2
        for n in range(N2):
            lo, hi = (tuple(fb[g, pl.ds(_yrow(2, n, part) + r, H), :] for part in range(2))
                      for r in (0, H))
            t = _tw(hi, n / 2, 1)
            zs = (_pack(lo[0] + t[0], lo[1] + t[1]), _pack(lo[0] - t[0], lo[1] - t[1]))
            for par in range(2):
                y_buf[g, pl.ds(n * YY + par * H, H), :] = jnp.dot(
                    pltpu.bitcast(inv_buf[n, rows(par, H // 2), :], bf16), zs[par],
                    preferred_element_type=f32)

    def out_copy(j):
        rs = pl.ds(OCH[j] * HB, (OCH[j + 1] - OCH[j]) * HB)
        return pltpu.make_async_copy(q_buf.at[rs], o_hbm.bitcast(u32).at[0, rs], osems.at[j])

    def gate(i, g, o):
        y = jnp.concatenate(
            [y_buf[g, pl.ds(i * (BM // 32) + (n // 2 + n % 2 * (N1 // 2) + h * YY), 8, stride=YY), :]
             for n in range(BM // N2) for h in (0, 8)], axis=0)
        xn = pltpu.bitcast(xn_buf[rows(i, HB), rows(g, 128)], bf16).astype(f32)
        q_buf[rows(i, HB), rows(g, 128)] = pltpu.bitcast((o + xn * y).astype(bf16), u32)

    def final(blocks):
        for i in blocks:
            for g in range(G):
                gate(i, g, acc[g, rows(i, BM), :])
                yield 150

    start(("q", 0))
    start(("w1", 0))
    for g in range(G):
        k_buf[g, pl.ds(0, 8), :] = jnp.zeros((8, 128), u32)
    b1_buf[...] = b1_ref[...].astype(f32).reshape(1, F)
    bt_buf[...] = jnp.broadcast_to(b1_buf[:, F - F % 128:], (128, F % 128)).T
    b2_buf[...] = b2_ref[...].astype(f32).reshape(1, D)
    wait(("q", 0))
    start(("q", 1))
    start(("w1", 1))
    _Fill(norm(0))(ALL)
    wait(("w1", 0))
    mm1(0, _Fill(()), 0, WCH[0], WCH[1])
    wait(("q", 1))
    start(("w1", 2), ("q", 2))
    _Fill(norm(1))(ALL)
    mm1(1, _Fill(()), 0, WCH[0], WCH[1])
    wait(("w1", 1))
    start(W2)
    for i in range(2):
        mm1(i, _Fill(()), 0, WCH[1], WCH[2])
    wait(("w1", 2))
    wait(("q", 2))
    start(("q", 3))
    fill = _Fill(norm(2, 3))
    for i in range(2):
        mm1(i, fill, FILLM, WCH[2], WCH[3])
    fill(ALL)
    start(("q", 4))
    wait(W2)
    wait(("q", 3))
    start(FWD, *conv_in(0, 1, 2))

    @pl.loop(0, 2)
    def _(i):
        @pl.when(i == 1)
        def _():
            wait(("q", 4))
            start(*conv_in(3, 4))

        fill = _Fill(norm(4 + i))
        mm2(i, fill, 40)
        fill(ALL)
        mm1(i + 2, fill, 0)

    wait(FWD, *conv_in(0, 1, 2))
    start(INV)
    _Fill(prep(-1))(ALL)
    for g in range(-1, G):
        if g == 1:
            wait(*conv_in(3, 4))
        stage1(g, prep(g + 1) if g + 1 < G else norm(6, 7), FILLB)

    @pl.loop(0, G - 1)
    def _(g):
        fill = _Fill(middle(g * NU, NU))
        mm2(g + 2, fill, FILL2)
        mm1(g + 4, fill, FILL1)
        fill(ALL)

    wait(INV)
    for g in range(G):
        inverse(g)

    fill = _Fill(final([i for i in range(NB - 2)]))
    mm2(NB - 2, fill, FILLE, last=True)
    fill(ALL)

    out_copy(0).start()
    mm2(NB - 1, _Fill(()), 0, last=True)
    out_copy(1).start()
    out_copy(0).wait()
    out_copy(1).wait()


OCH = (0, NB - 1, NB)
FILL1, FILL2 = 350, 115
ALL = 10**9
WCH = (0, 256, 768, F)
QCH = (0, 1, 2, 4, 5, NB)
W2, FWD, INV = ("mat", 0), ("mat", 1), ("mat", 2)
COPIES = ([("q", i) for i in range(5)] + [("w1", i) for i in range(3)] + [W2, FWD, INV]
          + [(kind, g) for g in range(G) for kind in ("ssm", "k", "v")])
NU = G * (N1 // 8) // 4
YY = N1 + 1
YP = N1 + 32


def _yrow(src, n, part):
    return ((src * N2 + n) * 2 + part) * YP + 8 * ((n // 4 + 2 * part) % 4)


NF = (F + 127) // 128
KH = 512
LC = 32
KP = 17


FILLB, FILLE, FILLM = 225, 70, 250


def _words(m):
    u = np.ascontiguousarray(m).view(np.uint16).astype(np.uint32)
    return u[..., 0::2, :] | (u[..., 1::2, :] << 16)


_FWD_P = _words(_FWD)
_INV_P = _words(_INV)


@jax.jit
def pallas_parallel_sum__ssm_conv_h3__dense_activation_gelu__prompt_kernel(
    A_q, A_k, A_v, A_shift_k, A_ssm_k, A_ssm_D, B_x, B_w1, B_b1, B_w2, B_b2,
):
    hbm = pl.BlockSpec(memory_space=pl.ANY)
    vmem = pl.BlockSpec(memory_space=pltpu.VMEM)
    return pl.pallas_call(
        _kernel,
        out_shape=jax.ShapeDtypeStruct((1, S, D), bf16),
        in_specs=[hbm, hbm, hbm, vmem, hbm, vmem, hbm, vmem, hbm, vmem, hbm, hbm,
                  pl.BlockSpec(memory_space=pltpu.SMEM)],
        out_specs=hbm,
        scratch_shapes=[
            pltpu.VMEM((S // 2, D), u32),
            pltpu.VMEM((G, S // 2 + 16, 128), u32),
            pltpu.VMEM((G, S // 2 + 8, 128), u32),
            pltpu.VMEM((D // 2, S), u32),
            pltpu.VMEM((F // 2, D), u32),
            pltpu.VMEM((F // 2, D), u32),
            pltpu.VMEM((N2, N1, N1), u32),
            pltpu.VMEM((N2, N1 // 2, N1), u32),
            pltpu.VMEM((G, KP * (N1 // 2 + 1), 128), u32),
            pltpu.VMEM((G, N2, N1 // 2, 128), u32),
            pltpu.VMEM((G, (N2 + 1) * YY + 24, 128), f32),
            pltpu.VMEM((S // 2, D), u32),
            pltpu.VMEM((S // 2, F), u32),
            pltpu.VMEM((G, S + 16, 128), f32),
            pltpu.VMEM((G, 6 * N2 * YP, 128), f32),
            pltpu.VMEM((1, F), f32),
            pltpu.VMEM((F % 128, 128), f32),
            pltpu.VMEM((1, D), f32),
            pltpu.SemaphoreType.DMA((len(COPIES),)),
            pltpu.SemaphoreType.DMA((2,)),
        ],
        compiler_params=pltpu.CompilerParams(vmem_limit_bytes=100 * 2**20),
    )(A_q, A_k, A_v, A_shift_k.T, A_ssm_k,
      A_ssm_D, B_w1.T, B_b1, B_w2, B_b2, _FWD_P, _INV_P, np.zeros((1,), np.int32))
```
